```python
import jax
import jax.numpy as jnp

def _softmax(x, axis=-1):
    return jax.nn.softmax(x, axis=axis)

def _gelu(x):
    return jax.nn.gelu(x, approximate=True)

def _silu(x):
    return jax.nn.silu(x)

def _sigmoid(x):
    return jax.nn.sigmoid(x)

def _layernorm(x, axis=-1, eps=1e-05):
    m = jnp.mean(x, axis=axis, keepdims=True)
    v = jnp.var(x, axis=axis, keepdims=True)
    return (x - m) / jnp.sqrt(v + eps)

def _scatter_add(tgt, idx, src, axis=0):
    return tgt.at[idx].add(src)

def _segment_sum(src, seg, n):
    return jax.ops.segment_sum(src, seg, n)

class _Rng:

    def __init__(self, key):
        self._k = key

    def _next(self):
        self._k, sub = jax.random.split(self._k)
        return sub

    def normal(self, shape):
        return jax.random.normal(self._next(), shape, dtype=jnp.bfloat16)

    def randint(self, lo, hi, shape):
        return jax.random.randint(self._next(), shape, lo, hi, dtype=jnp.int32)

    def uniform(self, shape, lo=0.0, hi=1.0):
        return jax.random.uniform(self._next(), shape, jnp.bfloat16, lo, hi)

    def permutation(self, n):
        return jax.random.permutation(self._next(), n)
kernel_name = 'parallel_sum__memory_aug_recurrent_mem_tr__moe_arch_mod__prompt'

def setup_inputs():
    _rng = _Rng(jax.random.key(int.from_bytes(__import__("os").urandom(4), "little")))
    _w = lambda a: (lambda t: t.astype(jnp.bfloat16) if jnp.issubdtype(t.dtype, jnp.floating) else t)(jnp.asarray(a))

    def _A_setup():
        B, S, Dm = (1, 2048, 1024)
        H, Dh = (32, 128)
        M, seg = (8, 32)
        seg = min(seg, S)
        S = S // seg * seg
        return {'x': _w((lambda *s: _rng.normal(s) * 0.05)(B, S, Dm)), 'mem0': _w((lambda *s: _rng.normal(s) * 0.05)(B, M, Dm)), 'Wq': _w((lambda *s: _rng.normal(s) * 0.05)(Dm, H, Dh) * Dm ** (-0.5)), 'Wk': _w((lambda *s: _rng.normal(s) * 0.05)(Dm, H, Dh) * Dm ** (-0.5)), 'Wv': _w((lambda *s: _rng.normal(s) * 0.05)(Dm, H, Dh) * Dm ** (-0.5)), 'Wo': _w((lambda *s: _rng.normal(s) * 0.05)(H, Dh, Dm) * (H * Dh) ** (-0.5)), 'seg_len': seg}
    _A_in = _A_setup()

    def _B_setup():
        B, S, D, F, C = (1, 2048, 1024, 3584, 2)
        return {'x': _w((lambda *s: _rng.normal(s) * 0.05)(B, S, D)), 'w_r': _w((lambda *s: _rng.normal(s) * 0.05)(D)), 'w_gate': _w((lambda *s: _rng.normal(s) * 0.05)(D, F)), 'w_up': _w((lambda *s: _rng.normal(s) * 0.05)(D, F)), 'w_down': _w((lambda *s: _rng.normal(s) * 0.05)(F, D))}
    _B_in = _B_setup()
    return {'A_x': _A_in['x'], 'A_mem0': _A_in['mem0'], 'A_Wq': _A_in['Wq'], 'A_Wk': _A_in['Wk'], 'A_Wv': _A_in['Wv'], 'A_Wo': _A_in['Wo'], 'A_seg_len': _A_in['seg_len'], 'B_x': _B_in['x'], 'B_w_r': _B_in['w_r'], 'B_w_gate': _B_in['w_gate'], 'B_w_up': _B_in['w_up'], 'B_w_down': _B_in['w_down']}

def reference(A_x, A_mem0, A_Wq, A_Wk, A_Wv, A_Wo, A_seg_len, B_x, B_w_r, B_w_gate, B_w_up, B_w_down):

    def _A_ref(x, mem0, Wq, Wk, Wv, Wo, seg_len):
        B, S, Dm = x.shape
        H, Dh = (Wq.shape[1], Wq.shape[2])
        M = mem0.shape[1]
        scale = Dh ** (-0.5)
        n_seg = S // seg_len
        L = M + seg_len
        idx = jnp.arange(L)
        mask = (idx[:, None] < M) | (idx[:, None] >= idx[None, :])
        mem = mem0
        outs = []
        for s in range(n_seg):
            xs = x[:, s * seg_len:(s + 1) * seg_len, :].copy()
            h = jnp.concatenate([mem, xs], axis=1)
            q = jnp.einsum('btd,dhe->bhte', h, Wq)
            k = jnp.einsum('btd,dhe->bhte', h, Wk)
            v = jnp.einsum('btd,dhe->bhte', h, Wv)
            scores = jnp.einsum('bhqe,bhke->bhqk', q, k) * scale
            scores = jnp.where(mask[None, None], scores, -1000000000.0)
            p = _softmax(scores, axis=-1)
            o = jnp.einsum('bhqk,bhke->bhqe', p, v)
            o = jnp.einsum('bhte,hed->btd', o, Wo)
            mem = o[:, :M, :].copy()
            outs.append(o[:, M:, :])
        return jnp.concatenate(outs, axis=1)

    def _B_ref(x, w_r, w_gate, w_up, w_down):
        B, S, D = x.shape
        C = 2
        r = x @ w_r
        idx = jnp.argsort(-r, axis=-1)[:, :C]
        idx_e = jnp.repeat(idx.reshape(B, C, 1), D, axis=2)
        x_sel = jnp.take_along_axis(x, idx_e, axis=1)
        g = _silu(x_sel @ w_gate)
        u = x_sel @ w_up
        y = g * u @ w_down
        r_sel = _sigmoid(jnp.take_along_axis(r, idx, axis=1))
        y = y * r_sel.reshape(B, C, 1)
        b_off = (jnp.arange(B) * S).reshape(B, 1)
        flat_idx = (idx + b_off).reshape(B * C)
        zero = (x * 0.0).reshape(B * S, D)
        upd = _scatter_add(zero, flat_idx, y.reshape(B * C, D), axis=0)
        return x + upd.reshape(B, S, D)
    x = A_x
    xn = _layernorm(x, axis=-1)
    return x + _A_ref(xn, A_mem0, A_Wq, A_Wk, A_Wv, A_Wo, A_seg_len) + _B_ref(xn, B_w_r, B_w_gate, B_w_up, B_w_down)
```

```python
import functools

import jax
import jax.numpy as jnp
import numpy as np
from jax import lax
from jax.experimental import pallas as pl
from jax.experimental.pallas import tpu as pltpu

F32 = jnp.float32
BF16 = jnp.bfloat16
U32 = jnp.uint32

PRE = 8
N_STAGE = 3
LN_EPS = 1e-05
MASKED = -1000000000.0
NUM_ROUTED = 2
LOW_HALF = np.uint32(0x0000FFFF)
HIGH_HALF = np.uint32(0xFFFF0000)


def _round_bf16(v):
    return v.astype(BF16).astype(F32)


def _layernorm_rows(x):
    xf = x.astype(F32)
    inv_n = 1.0 / xf.shape[-1]
    mean = jnp.sum(xf, axis=-1, keepdims=True) * inv_n
    cen = xf - mean
    var = jnp.sum(cen * cen, axis=-1, keepdims=True) * inv_n
    eps = jnp.full(var.shape, LN_EPS, BF16).astype(F32)
    std = _round_bf16(jnp.sqrt(_round_bf16(_round_bf16(var) + eps)))
    return _round_bf16(_round_bf16(xf - _round_bf16(mean)) / std)


def _matmul(a, b):
    return lax.dot_general(a, b, (((1,), (0,)), ((), ())), preferred_element_type=F32)


def _matmul_nt(a, b):
    return lax.dot_general(a, b, (((1,), (1,)), ((), ())), preferred_element_type=F32)


def _kernel(x_hbm, mem0_ref, wq_hbm, wk_hbm, wv_hbm, wo_hbm, wr_ref, wg_hbm, wu_hbm, wd_hbm,
            out_hbm,
            x_v, xn_pre, xn_rest, stage, wqkv, wo, pre, mem, out_v, wg, wu, wd, best_v, best_i,
            sem_x0, sem_in, sem_wo, sem_ffn, sem_out):
    n_seg, seg, dm = x_v.shape
    n_mem = mem.shape[0]
    n_pair = wqkv.shape[0]
    dh = wqkv.shape[2] // 6
    n_rows = n_mem + seg
    seg_per_pair = n_seg // n_pair
    wo_rows = wo.shape[0] // n_pair
    scale = dh ** -0.5

    w_in = [w.bitcast(U32) for w in (wq_hbm, wk_hbm, wv_hbm)]
    wo_in = wo_hbm.bitcast(U32)

    def pair_copies(j):
        slot = j % N_STAGE
        segs = pl.ds(j * seg_per_pair, seg_per_pair)
        rest = pl.ds(PRE, seg - PRE)
        copies = [pltpu.make_async_copy(w.at[:, j, :], stage.at[slot, i], sem_in.at[slot, i])
                  for i, w in enumerate(w_in)]
        copies.append(pltpu.make_async_copy(x_hbm.at[segs, rest, :], x_v.at[segs, rest, :],
                                            sem_in.at[slot, 3]))
        return copies

    def wo_copy(j):
        rows = pl.ds(j * wo_rows, wo_rows)
        return pltpu.make_async_copy(wo_in.at[rows, :], wo.at[rows, :], sem_wo.at[0])

    ffn_copies = [pltpu.make_async_copy(src.bitcast(U32), dst, sem_ffn.at[i])
                  for i, (src, dst) in enumerate(((wg_hbm, wg), (wu_hbm, wu), (wd_hbm, wd)))]

    def out_copy(s):
        return pltpu.make_async_copy(out_v.at[s], out_hbm.at[s], sem_out.at[0])

    x0_copy = pltpu.make_async_copy(x_hbm.at[:, pl.ds(0, PRE), :], x_v.at[:, pl.ds(0, PRE), :],
                                    sem_x0.at[0])
    x0_copy.start()
    for j in range(N_STAGE - 1):
        for c in pair_copies(j):
            c.start()

    mem[...] = mem0_ref[...].astype(F32)
    best_v[...] = jnp.full(best_v.shape, -jnp.inf, F32)
    best_i[...] = jnp.full(best_i.shape, n_seg * seg, jnp.int32)
    x0_copy.wait()

    def norm_first_rows(i, carry):
        segs = pl.ds(i * 8, 8)
        rows = x_v[segs, pl.ds(0, PRE), :].astype(F32).reshape(8 * PRE, dm)
        xn_pre[pl.ds(pl.multiple_of(i * 8 * PRE, 8 * PRE), 8 * PRE), :] = _layernorm_rows(rows)
        return carry

    lax.fori_loop(0, n_seg // 8, norm_first_rows, 0)

    def project_pair(j, carry):
        @pl.when(j + N_STAGE - 1 < n_pair)
        def _():
            for c in pair_copies(j + N_STAGE - 1):
                c.start()

        wo_copy(j).start()
        for c in pair_copies(j):
            c.wait()

        slot = j % N_STAGE
        lhs = xn_pre[...]
        for i in range(3):
            even = stage[slot, i, pl.ds(0, dm // 2, stride=2), :]
            odd = stage[slot, i, pl.ds(1, dm // 2, stride=2), :]
            heads = ((even & LOW_HALF) | (odd << 16), (even >> 16) | (odd & HIGH_HALF))
            for p in range(2):
                cols = pl.ds((3 * p + i) * dh, dh)
                wqkv[j, :, cols] = heads[p]
                pre[j, :, cols] = _matmul(lhs, pltpu.bitcast(heads[p], BF16))

        w_r = jnp.broadcast_to(wr_ref[...].astype(F32).reshape(1, dm), (8, dm))
        v1, v2, i1, i2 = best_v[0], best_v[1], best_i[0], best_i[1]
        sub = lax.broadcasted_iota(jnp.int32, v1.shape, 0)
        for t in range(seg_per_pair):
            s = j * seg_per_pair + t
            rest = _layernorm_rows(x_v[s, pl.ds(PRE, seg - PRE), :])
            xn_rest[s] = rest
            first = xn_pre[pl.ds(pl.multiple_of(s * PRE, PRE), PRE), :]
            rows = jnp.concatenate([first, rest], axis=0)
            for g in range(seg // 8):
                r = jnp.sum(rows[g * 8:(g + 1) * 8] * w_r, axis=-1, keepdims=True)
                r = jnp.broadcast_to(_round_bf16(r), v1.shape)
                idx = sub + (s * seg + g * 8)
                gt1, gt2 = r > v1, r > v2
                v2 = jnp.where(gt1, v1, jnp.where(gt2, r, v2))
                i2 = jnp.where(gt1, i1, jnp.where(gt2, idx, i2))
                v1 = jnp.where(gt1, r, v1)
                i1 = jnp.where(gt1, idx, i1)
        best_v[0], best_v[1], best_i[0], best_i[1] = v1, v2, i1, i2
        return carry

    lax.fori_loop(0, n_pair, project_pair, 0)

    for c in ffn_copies:
        c.start()

    vals = jnp.concatenate([best_v[0], best_v[1]], axis=0)
    idxs = jnp.concatenate([best_i[0], best_i[1]], axis=0)
    routed = []
    for _ in range(NUM_ROUTED):
        top = jnp.max(vals, axis=0, keepdims=True)
        pick = jnp.min(jnp.where(vals == top, idxs, n_seg * seg), axis=0, keepdims=True)
        vals = jnp.where(idxs == pick, -jnp.inf, vals)
        routed.append((jnp.clip(jnp.min(pick), 0, n_seg * seg - 1), top))
    routed_seg = [tok // seg for tok, _ in routed]

    pltpu.make_async_copy(wo_in, wo, sem_wo.at[0]).wait()

    row = lax.broadcasted_iota(jnp.int32, (n_rows, n_rows), 0)
    col = lax.broadcasted_iota(jnp.int32, (n_rows, n_rows), 1)
    visible = (row < n_mem) | (row >= col)

    def step(s, carry):
        first_rows = pl.ds(pl.multiple_of(s * PRE, PRE), PRE)
        rest = xn_rest[s]
        lhs = jnp.concatenate([mem[...], rest], axis=0).astype(BF16)
        qkv, probs, heads = {}, {}, {}

        def project(j):
            r = _matmul(lhs, pltpu.bitcast(wqkv[j], BF16))
            qkv[j] = jnp.concatenate([r[:n_mem], pre[j, first_rows, :], r[n_mem:]], axis=0)

        def part(j, p, i):
            return qkv[j][:, (3 * p + i) * dh:(3 * p + i + 1) * dh]

        def scores(j):
            for p in range(2):
                sc = _matmul_nt(part(j, p, 0), part(j, p, 1).astype(BF16)) * scale
                sc = jnp.where(visible, sc, MASKED)
                e = jnp.exp(sc - jnp.max(sc, axis=-1, keepdims=True))
                probs[j, p] = (e, jnp.sum(e, axis=-1, keepdims=True))

        def mix(j):
            for p in range(2):
                e, denom = probs[j, p]
                heads[2 * j + p] = _matmul(e, part(j, p, 2).astype(BF16)) / denom

        def out_proj(h0, h1):
            o = jnp.concatenate([heads[h] for h in range(h0, h1)], axis=1)
            return _matmul(o, pltpu.bitcast(wo[h0 * dh // 2:h1 * dh // 2, :], BF16))

        for t in range(n_pair + 2):
            if t < n_pair:
                project(t)
            if t == n_pair:
                o = out_proj(0, n_pair)
            if t >= 2:
                mix(t - 2)
            if 1 <= t <= n_pair:
                scores(t - 1)
        o = o + out_proj(n_pair, 2 * n_pair)

        mem[...] = o[:n_mem]
        xn = jnp.concatenate([xn_pre[first_rows, :], rest], axis=0)
        out_v[s] = ((x_v[s].astype(F32) + o[n_mem:]) + xn).astype(BF16)

        @pl.when((s != routed_seg[0]) & (s != routed_seg[1]))
        def _():
            out_copy(s).start()

        return carry

    lax.fori_loop(0, n_seg, step, 0)

    seg_row = lax.broadcasted_iota(jnp.int32, (seg, dm), 0)
    sel_row = lax.broadcasted_iota(jnp.int32, (8, dm), 0)
    x_sel = jnp.zeros((8, dm), F32)
    gate = jnp.zeros((8, 1), F32)
    for c, (tok, score) in enumerate(routed):
        s = routed_seg[c]
        xn = jnp.concatenate([xn_pre[pl.ds(pl.multiple_of(s * PRE, PRE), PRE), :], xn_rest[s]], axis=0)
        picked = jnp.sum(jnp.where(seg_row == tok - s * seg, xn, 0.0), axis=0, keepdims=True)
        x_sel = jnp.where(sel_row == c, picked, x_sel)
        gate = jnp.where(sel_row[:, :1] == c, jax.nn.sigmoid(score[:, :1]), gate)

    ffn_copies[0].wait()
    g = _matmul(x_sel, pltpu.bitcast(wg[...], BF16))
    ffn_copies[1].wait()
    u = _matmul(x_sel, pltpu.bitcast(wu[...], BF16))
    ffn_copies[2].wait()
    y = _matmul(g * jax.nn.sigmoid(g) * u, pltpu.bitcast(wd[...], BF16)) * gate

    for c, (tok, _) in enumerate(routed):
        s = routed_seg[c]
        upd = jnp.where(seg_row == tok - s * seg, y[c:c + 1], 0.0)
        out_v[s] = (out_v[s].astype(F32) + upd).astype(BF16)

    out_copy(routed_seg[0]).start()

    @pl.when(routed_seg[1] != routed_seg[0])
    def _():
        out_copy(routed_seg[1]).start()

    pltpu.make_async_copy(out_v, out_hbm, sem_out.at[0]).wait()


@functools.partial(jax.jit, static_argnames=("A_seg_len",))
def pallas_parallel_sum__memory_aug_recurrent_mem_tr__moe_arch_mod__prompt_kernel(
    A_x: jax.Array,
    A_mem0: jax.Array,
    A_Wq: jax.Array,
    A_Wk: jax.Array,
    A_Wv: jax.Array,
    A_Wo: jax.Array,
    A_seg_len: int,
    B_x: jax.Array,
    B_w_r: jax.Array,
    B_w_gate: jax.Array,
    B_w_up: jax.Array,
    B_w_down: jax.Array,
):
    del B_x
    batch, n_tok, dm = A_x.shape
    _, n_head, dh = A_Wq.shape
    n_mem = A_mem0.shape[1]
    seg = A_seg_len
    n_seg = n_tok // seg
    n_pair = n_head // 2
    ff = B_w_gate.shape[1]
    assert batch == 1 and n_mem == 8 and dh == 128 and seg % 16 == 0 and n_tok == n_seg * seg
    assert n_seg % n_pair == 0 and n_seg % 8 == 0

    hbm = pl.BlockSpec(memory_space=pl.ANY)
    vmem = pl.BlockSpec(memory_space=pltpu.VMEM)
    out = pl.pallas_call(
        _kernel,
        out_shape=jax.ShapeDtypeStruct((n_seg, seg, dm), A_x.dtype),
        in_specs=[hbm, vmem, hbm, hbm, hbm, hbm, vmem, hbm, hbm, hbm],
        out_specs=hbm,
        scratch_shapes=[
            pltpu.VMEM((n_seg, seg, dm), BF16),
            pltpu.VMEM((n_seg * PRE, dm), F32),
            pltpu.VMEM((n_seg, seg - PRE, dm), F32),
            pltpu.VMEM((N_STAGE, 3, dm, dh), U32),
            pltpu.VMEM((n_pair, dm // 2, 6 * dh), U32),
            pltpu.VMEM((n_head * dh // 2, dm), U32),
            pltpu.VMEM((n_pair, n_seg * PRE, 6 * dh), F32),
            pltpu.VMEM((n_mem, dm), F32),
            pltpu.VMEM((n_seg, seg, dm), BF16),
            pltpu.VMEM((dm // 2, ff), U32),
            pltpu.VMEM((dm // 2, ff), U32),
            pltpu.VMEM((ff // 2, dm), U32),
            pltpu.VMEM((NUM_ROUTED, 8, 128), F32),
            pltpu.VMEM((NUM_ROUTED, 8, 128), jnp.int32),
            pltpu.SemaphoreType.DMA((1,)),
            pltpu.SemaphoreType.DMA((N_STAGE, 4)),
            pltpu.SemaphoreType.DMA((1,)),
            pltpu.SemaphoreType.DMA((3,)),
            pltpu.SemaphoreType.DMA((1,)),
        ],
        compiler_params=pltpu.CompilerParams(vmem_limit_bytes=120 * 1024 * 1024),
        name="rmt_mod_fused",
    )(
        A_x.reshape(n_seg, seg, dm),
        A_mem0.reshape(n_mem, dm),
        A_Wq,
        A_Wk,
        A_Wv,
        A_Wo.reshape(n_head * dh, dm),
        B_w_r,
        B_w_gate,
        B_w_up,
        B_w_down,
    )
    return out.reshape(batch, n_tok, dm)
```

```python
import functools

import jax
import jax.numpy as jnp
import numpy as np
from jax import lax
from jax.experimental import pallas as pl
from jax.experimental.pallas import tpu as pltpu

F32 = jnp.float32
BF16 = jnp.bfloat16
U32 = jnp.uint32

PRE = 8
N_STAGE = 3
STEP_UNROLL = 2
LN_EPS = 1e-05
MASKED = -1000000000.0
NUM_ROUTED = 2
LOW_HALF = np.uint32(0x0000FFFF)
HIGH_HALF = np.uint32(0xFFFF0000)


def _round_bf16(v):
    return v.astype(BF16).astype(F32)


def _layernorm_rows(x):
    xf = x.astype(F32)
    inv_n = 1.0 / xf.shape[-1]
    mean = jnp.sum(xf, axis=-1, keepdims=True) * inv_n
    cen = xf - mean
    var = jnp.sum(cen * cen, axis=-1, keepdims=True) * inv_n
    eps = jnp.full(var.shape, LN_EPS, BF16).astype(F32)
    std = _round_bf16(jnp.sqrt(_round_bf16(_round_bf16(var) + eps)))
    return _round_bf16(_round_bf16(xf - _round_bf16(mean)) / std)


def _matmul(a, b):
    return lax.dot_general(a, b, (((1,), (0,)), ((), ())), preferred_element_type=F32)


def _matmul_nt(a, b):
    return lax.dot_general(a, b, (((1,), (1,)), ((), ())), preferred_element_type=F32)


def _kernel(x_hbm, mem0_ref, wq_hbm, wk_hbm, wv_hbm, wo_hbm, wr_ref, wg_hbm, wu_hbm, wd_hbm,
            out_hbm,
            x_v, xn_pre, xn_rest, stage, wqkv, wo, pre, mem, acc, out_v, wg, wu, wd, best_v, best_i,
            sem_x0, sem_in, sem_wo, sem_ffn, sem_out):
    n_seg, seg, dm = x_v.shape
    n_mem = mem.shape[0]
    n_pair = wqkv.shape[0]
    dh = wqkv.shape[2] // 6
    n_rows = n_mem + seg
    seg_per_pair = n_seg // n_pair
    wo_rows = wo.shape[0] // n_pair
    scale = dh ** -0.5

    w_in = [w.bitcast(U32) for w in (wq_hbm, wk_hbm, wv_hbm)]
    wo_in = wo_hbm.bitcast(U32)

    def pair_copies(j):
        slot = j % N_STAGE
        segs = pl.ds(j * seg_per_pair, seg_per_pair)
        rest = pl.ds(PRE, seg - PRE)
        copies = [pltpu.make_async_copy(w.at[:, j, :], stage.at[slot, i], sem_in.at[slot, i])
                  for i, w in enumerate(w_in)]
        copies.append(pltpu.make_async_copy(x_hbm.at[segs, rest, :], x_v.at[segs, rest, :],
                                            sem_in.at[slot, 3]))
        return copies

    def wo_copy(j):
        rows = pl.ds(j * wo_rows, wo_rows)
        return pltpu.make_async_copy(wo_in.at[rows, :], wo.at[rows, :], sem_wo.at[0])

    ffn_copies = [pltpu.make_async_copy(src.bitcast(U32), dst, sem_ffn.at[i])
                  for i, (src, dst) in enumerate(((wg_hbm, wg), (wu_hbm, wu), (wd_hbm, wd)))]

    def out_copy(s):
        return pltpu.make_async_copy(out_v.at[s], out_hbm.at[s], sem_out.at[0])

    x0_copy = pltpu.make_async_copy(x_hbm.at[:, pl.ds(0, PRE), :], x_v.at[:, pl.ds(0, PRE), :],
                                    sem_x0.at[0])
    x0_copy.start()
    for j in range(N_STAGE - 1):
        for c in pair_copies(j):
            c.start()

    mem[...] = mem0_ref[...].astype(F32)
    best_v[...] = jnp.full(best_v.shape, -jnp.inf, F32)
    best_i[...] = jnp.full(best_i.shape, n_seg * seg, jnp.int32)
    x0_copy.wait()

    def norm_first_rows(i, carry):
        segs = pl.ds(i * 8, 8)
        rows = x_v[segs, pl.ds(0, PRE), :].astype(F32).reshape(8 * PRE, dm)
        xn_pre[pl.ds(pl.multiple_of(i * 8 * PRE, 8 * PRE), 8 * PRE), :] = _layernorm_rows(rows)
        return carry

    lax.fori_loop(0, n_seg // 8, norm_first_rows, 0)

    def project_pair(j, carry):
        @pl.when(j + N_STAGE - 1 < n_pair)
        def _():
            for c in pair_copies(j + N_STAGE - 1):
                c.start()

        wo_copy(j).start()
        for c in pair_copies(j):
            c.wait()

        slot = j % N_STAGE
        lhs = xn_pre[...]
        for i in range(3):
            even = stage[slot, i, pl.ds(0, dm // 2, stride=2), :]
            odd = stage[slot, i, pl.ds(1, dm // 2, stride=2), :]
            heads = ((even & LOW_HALF) | (odd << 16), (even >> 16) | (odd & HIGH_HALF))
            for p in range(2):
                cols = pl.ds((3 * p + i) * dh, dh)
                wqkv[j, :, cols] = heads[p]
                pre[j, :, cols] = _matmul(lhs, pltpu.bitcast(heads[p], BF16))

        w_r = jnp.broadcast_to(wr_ref[...].astype(F32).reshape(1, dm), (8, dm))
        v1, v2, i1, i2 = best_v[0], best_v[1], best_i[0], best_i[1]
        sub = lax.broadcasted_iota(jnp.int32, v1.shape, 0)
        for t in range(seg_per_pair):
            s = j * seg_per_pair + t
            rest = _layernorm_rows(x_v[s, pl.ds(PRE, seg - PRE), :])
            xn_rest[s] = rest
            first = xn_pre[pl.ds(pl.multiple_of(s * PRE, PRE), PRE), :]
            rows = jnp.concatenate([first, rest], axis=0)
            for g in range(seg // 8):
                r = jnp.sum(rows[g * 8:(g + 1) * 8] * w_r, axis=-1, keepdims=True)
                r = jnp.broadcast_to(_round_bf16(r), v1.shape)
                idx = sub + (s * seg + g * 8)
                gt1, gt2 = r > v1, r > v2
                v2 = jnp.where(gt1, v1, jnp.where(gt2, r, v2))
                i2 = jnp.where(gt1, i1, jnp.where(gt2, idx, i2))
                v1 = jnp.where(gt1, r, v1)
                i1 = jnp.where(gt1, idx, i1)
        best_v[0], best_v[1], best_i[0], best_i[1] = v1, v2, i1, i2
        return carry

    lax.fori_loop(0, n_pair, project_pair, 0)

    for c in ffn_copies:
        c.start()

    vals = jnp.concatenate([best_v[0], best_v[1]], axis=0)
    idxs = jnp.concatenate([best_i[0], best_i[1]], axis=0)
    routed = []
    for _ in range(NUM_ROUTED):
        top = jnp.max(vals, axis=0, keepdims=True)
        pick = jnp.min(jnp.where(vals == top, idxs, n_seg * seg), axis=0, keepdims=True)
        vals = jnp.where(idxs == pick, -jnp.inf, vals)
        routed.append((jnp.clip(jnp.min(pick), 0, n_seg * seg - 1), top))
    routed_seg = [tok // seg for tok, _ in routed]

    pltpu.make_async_copy(wo_in, wo, sem_wo.at[0]).wait()

    row = lax.broadcasted_iota(jnp.int32, (n_rows, n_rows), 0)
    col = lax.broadcasted_iota(jnp.int32, (n_rows, n_rows), 1)
    visible = (row < n_mem) | (row >= col)

    def step(s, memory):
        first_rows = pl.ds(pl.multiple_of(s * PRE, PRE), PRE)
        rest = xn_rest[s]
        lhs = jnp.concatenate([memory, rest], axis=0).astype(BF16)
        qkv, probs, heads = {}, {}, {}

        def project(j):
            r = _matmul(lhs, pltpu.bitcast(wqkv[j], BF16))
            qkv[j] = jnp.concatenate([r[:n_mem], pre[j, first_rows, :], r[n_mem:]], axis=0)

        def part(j, p, i):
            return qkv[j][:, (3 * p + i) * dh:(3 * p + i + 1) * dh]

        def scores(j):
            for p in range(2):
                sc = _matmul_nt(part(j, p, 0), part(j, p, 1).astype(BF16)) * scale
                sc = jnp.where(visible, sc, MASKED)
                e = jnp.exp(sc - jnp.max(sc, axis=-1, keepdims=True))
                probs[j, p] = (e, jnp.sum(e, axis=-1, keepdims=True))

        def mix(j):
            for p in range(2):
                e, denom = probs[j, p]
                heads[2 * j + p] = _matmul(e, part(j, p, 2).astype(BF16)) / denom

        def out_proj(quarter):
            h0, h1 = quarter * n_pair // 2, (quarter + 1) * n_pair // 2
            o = jnp.concatenate([heads[h] for h in range(h0, h1)], axis=1)
            return _matmul(o, pltpu.bitcast(wo[h0 * dh // 2:h1 * dh // 2, :], BF16))

        for j in range(n_pair):
            project(j)
            if j >= 2:
                mix(j - 2)
            if j >= 1:
                scores(j - 1)
        acc[...] = out_proj(0)
        mix(n_pair - 2)
        scores(n_pair - 1)
        acc[...] += out_proj(1)
        mix(n_pair - 1)
        acc[...] += out_proj(2)
        o = acc[...] + out_proj(3)

        xn = jnp.concatenate([xn_pre[first_rows, :], rest], axis=0)
        out_v[s] = ((x_v[s].astype(F32) + o[n_mem:]) + xn).astype(BF16)
        return o[:n_mem]

    def steps(i, carry):
        memory = mem[...]
        for u in range(STEP_UNROLL):
            memory = step(i * STEP_UNROLL + u, memory)
        mem[...] = memory
        for u in range(STEP_UNROLL):
            s = i * STEP_UNROLL + u

            @pl.when((s != routed_seg[0]) & (s != routed_seg[1]))
            def _():
                out_copy(s).start()

        return carry

    lax.fori_loop(0, n_seg // STEP_UNROLL, steps, 0)

    seg_row = lax.broadcasted_iota(jnp.int32, (seg, dm), 0)
    sel_row = lax.broadcasted_iota(jnp.int32, (8, dm), 0)
    x_sel = jnp.zeros((8, dm), F32)
    gate = jnp.zeros((8, 1), F32)
    for c, (tok, score) in enumerate(routed):
        s = routed_seg[c]
        xn = jnp.concatenate([xn_pre[pl.ds(pl.multiple_of(s * PRE, PRE), PRE), :], xn_rest[s]], axis=0)
        picked = jnp.sum(jnp.where(seg_row == tok - s * seg, xn, 0.0), axis=0, keepdims=True)
        x_sel = jnp.where(sel_row == c, picked, x_sel)
        gate = jnp.where(sel_row[:, :1] == c, jax.nn.sigmoid(score[:, :1]), gate)

    ffn_copies[0].wait()
    g = _matmul(x_sel, pltpu.bitcast(wg[...], BF16))
    ffn_copies[1].wait()
    u = _matmul(x_sel, pltpu.bitcast(wu[...], BF16))
    ffn_copies[2].wait()
    y = _matmul(g * jax.nn.sigmoid(g) * u, pltpu.bitcast(wd[...], BF16)) * gate

    for c, (tok, _) in enumerate(routed):
        s = routed_seg[c]
        upd = jnp.where(seg_row == tok - s * seg, y[c:c + 1], 0.0)
        out_v[s] = (out_v[s].astype(F32) + upd).astype(BF16)

    out_copy(routed_seg[0]).start()

    @pl.when(routed_seg[1] != routed_seg[0])
    def _():
        out_copy(routed_seg[1]).start()

    pltpu.make_async_copy(out_v, out_hbm, sem_out.at[0]).wait()


@functools.partial(jax.jit, static_argnames=("A_seg_len",))
def pallas_parallel_sum__memory_aug_recurrent_mem_tr__moe_arch_mod__prompt_kernel(
    A_x: jax.Array,
    A_mem0: jax.Array,
    A_Wq: jax.Array,
    A_Wk: jax.Array,
    A_Wv: jax.Array,
    A_Wo: jax.Array,
    A_seg_len: int,
    B_x: jax.Array,
    B_w_r: jax.Array,
    B_w_gate: jax.Array,
    B_w_up: jax.Array,
    B_w_down: jax.Array,
):
    del B_x
    batch, n_tok, dm = A_x.shape
    _, n_head, dh = A_Wq.shape
    n_mem = A_mem0.shape[1]
    seg = A_seg_len
    n_seg = n_tok // seg
    n_pair = n_head // 2
    ff = B_w_gate.shape[1]
    assert batch == 1 and n_mem == 8 and dh == 128 and seg % 16 == 0 and n_tok == n_seg * seg
    assert n_seg % n_pair == 0 and n_seg % 8 == 0

    hbm = pl.BlockSpec(memory_space=pl.ANY)
    vmem = pl.BlockSpec(memory_space=pltpu.VMEM)
    out = pl.pallas_call(
        _kernel,
        out_shape=jax.ShapeDtypeStruct((n_seg, seg, dm), A_x.dtype),
        in_specs=[hbm, vmem, hbm, hbm, hbm, hbm, vmem, hbm, hbm, hbm],
        out_specs=hbm,
        scratch_shapes=[
            pltpu.VMEM((n_seg, seg, dm), BF16),
            pltpu.VMEM((n_seg * PRE, dm), F32),
            pltpu.VMEM((n_seg, seg - PRE, dm), F32),
            pltpu.VMEM((N_STAGE, 3, dm, dh), U32),
            pltpu.VMEM((n_pair, dm // 2, 6 * dh), U32),
            pltpu.VMEM((n_head * dh // 2, dm), U32),
            pltpu.VMEM((n_pair, n_seg * PRE, 6 * dh), F32),
            pltpu.VMEM((n_mem, dm), F32),
            pltpu.VMEM((n_mem + seg, dm), F32),
            pltpu.VMEM((n_seg, seg, dm), BF16),
            pltpu.VMEM((dm // 2, ff), U32),
            pltpu.VMEM((dm // 2, ff), U32),
            pltpu.VMEM((ff // 2, dm), U32),
            pltpu.VMEM((NUM_ROUTED, 8, 128), F32),
            pltpu.VMEM((NUM_ROUTED, 8, 128), jnp.int32),
            pltpu.SemaphoreType.DMA((1,)),
            pltpu.SemaphoreType.DMA((N_STAGE, 4)),
            pltpu.SemaphoreType.DMA((1,)),
            pltpu.SemaphoreType.DMA((3,)),
            pltpu.SemaphoreType.DMA((1,)),
        ],
        compiler_params=pltpu.CompilerParams(vmem_limit_bytes=120 * 1024 * 1024),
        name="rmt_mod_fused",
    )(
        A_x.reshape(n_seg, seg, dm),
        A_mem0.reshape(n_mem, dm),
        A_Wq,
        A_Wk,
        A_Wv,
        A_Wo.reshape(n_head * dh, dm),
        B_w_r,
        B_w_gate,
        B_w_up,
        B_w_down,
    )
    return out.reshape(batch, n_tok, dm)
```

```python
import functools

import jax
import jax.numpy as jnp
import numpy as np
from jax import lax
from jax.experimental import pallas as pl
from jax.experimental.pallas import tpu as pltpu

F32 = jnp.float32
BF16 = jnp.bfloat16
U32 = jnp.uint32

PRE = 8
X0_CHUNKS = 4
N_STAGE = 3
PAIR_UNROLL = 3
STEP_UNROLL = 4
FF_CHUNK = 256
LN_EPS = 1e-05
MASKED = -1000000000.0
NUM_ROUTED = 2
LOW_HALF = np.uint32(0x0000FFFF)
HIGH_HALF = np.uint32(0xFFFF0000)


def _round_bf16(v):
    return v.astype(BF16).astype(F32)


def _layernorm_rows(x):
    xf = x.astype(F32)
    inv_n = 1.0 / xf.shape[-1]
    mean = jnp.sum(xf, axis=-1, keepdims=True) * inv_n
    cen = xf - mean
    var = jnp.sum(cen * cen, axis=-1, keepdims=True) * inv_n
    eps = jnp.full(var.shape, LN_EPS, BF16).astype(F32)
    std = _round_bf16(jnp.sqrt(_round_bf16(_round_bf16(var) + eps)))
    return _round_bf16(_round_bf16(xf - _round_bf16(mean)) / std)


def _matmul(a, b):
    return lax.dot_general(a, b, (((1,), (0,)), ((), ())), preferred_element_type=F32)


def _matmul_nt(a, b):
    return lax.dot_general(a, b, (((1,), (1,)), ((), ())), preferred_element_type=F32)


def _weights(words):
    return pltpu.bitcast(words, BF16)


def _kernel(x_hbm, mem0_ref, wq_hbm, wk_hbm, wv_hbm, wo_hbm, wr_ref, wg_hbm, wu_hbm, wd_hbm,
            out_hbm,
            x_v, xn_pre, xn_rest, stage, wqkv, wo, pre, mem, acc, acc_first, out_v,
            wg, wu, wd, x_sel, gate_up, hidden, y_acc, best_v, best_i,
            sem_x0, sem_in, sem_wo, sem_ffn, sem_out):
    n_seg, seg, dm = x_v.shape
    n_mem = mem.shape[0]
    n_pair = wqkv.shape[0]
    dh = wqkv.shape[2] // 6
    n_rows = n_mem + seg
    n_tok = n_seg * seg
    ff = wd_hbm.shape[0]
    seg_per_pair = n_seg // n_pair
    wo_rows = wo.shape[0] // n_pair
    scale = dh ** -0.5

    w_in = [w.bitcast(U32) for w in (wq_hbm, wk_hbm, wv_hbm)]
    wo_in = wo_hbm.bitcast(U32)

    def x0_copy(c):
        segs = pl.ds(c * n_seg // X0_CHUNKS, n_seg // X0_CHUNKS)
        return pltpu.make_async_copy(x_hbm.at[segs, pl.ds(0, PRE), :], x_v.at[segs, pl.ds(0, PRE), :],
                                     sem_x0.at[c])

    def w_copy(j, i):
        slot = j % N_STAGE
        return pltpu.make_async_copy(w_in[i].at[:, j, :], stage.at[slot, i], sem_in.at[slot, i])

    def x_copy(j):
        segs = pl.ds(j * seg_per_pair, seg_per_pair)
        rest = pl.ds(PRE, seg - PRE)
        return pltpu.make_async_copy(x_hbm.at[segs, rest, :], x_v.at[segs, rest, :],
                                     sem_in.at[j % N_STAGE, 3])

    def start_pair(j):
        for i in range(3):
            w_copy(j, i).start()
        x_copy(j).start()

    def wo_copy(j):
        rows = pl.ds(j * wo_rows, wo_rows)
        return pltpu.make_async_copy(wo_in.at[rows, :], wo.at[rows, :], sem_wo.at[0])

    ffn_copies = [
        pltpu.make_async_copy(wg_hbm.bitcast(U32), wg.at[:, pl.ds(0, ff)], sem_ffn.at[0]),
        pltpu.make_async_copy(wu_hbm.bitcast(U32), wu.at[:, pl.ds(0, ff)], sem_ffn.at[1]),
        pltpu.make_async_copy(wd_hbm.bitcast(U32), wd.at[pl.ds(0, ff // 2), :], sem_ffn.at[2]),
    ]

    def out_copy(s):
        return pltpu.make_async_copy(out_v.at[s], out_hbm.at[s], sem_out.at[0])

    def first_rows(s):
        return pl.ds(pl.multiple_of(s * PRE, PRE), PRE)

    for c in range(X0_CHUNKS):
        x0_copy(c).start()
        if c < 3:
            w_copy(0, c).start()
    x_copy(0).start()
    for j in range(1, N_STAGE - 1):
        start_pair(j)

    mem[...] = mem0_ref[...].astype(F32)
    best_v[...] = jnp.full(best_v.shape, -jnp.inf, F32)
    best_i[...] = jnp.full(best_i.shape, n_tok, jnp.int32)

    def split_heads(j, i):
        slot = j % N_STAGE
        even = stage[slot, i, pl.ds(0, dm // 2, stride=2), :]
        odd = stage[slot, i, pl.ds(1, dm // 2, stride=2), :]
        heads = ((even & LOW_HALF) | (odd << 16), (even >> 16) | (odd & HIGH_HALF))
        for p in range(2):
            wqkv[j, :, pl.ds((3 * p + i) * dh, dh)] = heads[p]
        return heads

    def route_segments(j):
        w_r = jnp.broadcast_to(wr_ref[...].astype(F32).reshape(1, dm), (8, dm))
        v1, v2, i1, i2 = best_v[0], best_v[1], best_i[0], best_i[1]
        sub = lax.broadcasted_iota(jnp.int32, v1.shape, 0)
        for t in range(seg_per_pair):
            s = j * seg_per_pair + t
            rest = _layernorm_rows(x_v[s, pl.ds(PRE, seg - PRE), :])
            xn_rest[s] = rest
            rows = jnp.concatenate([xn_pre[first_rows(s), :], rest], axis=0)
            for g in range(seg // 8):
                r = jnp.sum(rows[g * 8:(g + 1) * 8] * w_r, axis=-1, keepdims=True)
                r = jnp.broadcast_to(_round_bf16(r), v1.shape)
                idx = sub + (s * seg + g * 8)
                gt1, gt2 = r > v1, r > v2
                v2 = jnp.where(gt1, v1, jnp.where(gt2, r, v2))
                i2 = jnp.where(gt1, i1, jnp.where(gt2, idx, i2))
                v1 = jnp.where(gt1, r, v1)
                i1 = jnp.where(gt1, idx, i1)
        best_v[0], best_v[1], best_i[0], best_i[1] = v1, v2, i1, i2

    def project_first_rows(j, i, rows=slice(None), heads=None):
        heads = split_heads(j, i) if heads is None else heads
        for p in range(2):
            pre[j, rows, pl.ds((3 * p + i) * dh, dh)] = _matmul(xn_pre[rows, :], _weights(heads[p]))

    start_pair(N_STAGE - 1)
    wo_copy(0).start()
    chunk_segs = n_seg // X0_CHUNKS
    chunk_rows = chunk_segs * PRE

    def norm_chunk(c):
        x0_copy(c).wait()
        rows = x_v[pl.ds(c * chunk_segs, chunk_segs), pl.ds(0, PRE), :].astype(F32)
        xn_pre[pl.ds(c * chunk_rows, chunk_rows), :] = _layernorm_rows(rows.reshape(chunk_rows, dm))

    norm_chunk(0)
    w_copy(0, 0).wait()
    q_heads = split_heads(0, 0)
    for c in range(X0_CHUNKS):
        if c + 1 < X0_CHUNKS:
            norm_chunk(c + 1)
        project_first_rows(0, 0, pl.ds(c * chunk_rows, chunk_rows), q_heads)
    for i in (1, 2):
        w_copy(0, i).wait()
    x_copy(0).wait()
    for i in (1, 2):
        project_first_rows(0, i)
    route_segments(0)

    def project_pairs(t, carry):
        for u in range(PAIR_UNROLL):
            j = 1 + t * PAIR_UNROLL + u

            @pl.when(j + N_STAGE - 1 < n_pair)
            def _():
                start_pair(j + N_STAGE - 1)

            wo_copy(j).start()
            for i in range(3):
                w_copy(j, i).wait()
            x_copy(j).wait()
            for i in range(3):
                project_first_rows(j, i)
            route_segments(j)
        return carry

    lax.fori_loop(0, (n_pair - 1) // PAIR_UNROLL, project_pairs, 0)

    wg[:, pl.ds(ff, FF_CHUNK)] = jnp.zeros((dm // 2, FF_CHUNK), U32)
    wu[:, pl.ds(ff, FF_CHUNK)] = jnp.zeros((dm // 2, FF_CHUNK), U32)
    wd[pl.ds(ff // 2, FF_CHUNK // 2), :] = jnp.zeros((FF_CHUNK // 2, dm), U32)
    for c in ffn_copies:
        c.start()

    vals = jnp.concatenate([best_v[0], best_v[1]], axis=0)
    idxs = jnp.concatenate([best_i[0], best_i[1]], axis=0)
    seg_row = lax.broadcasted_iota(jnp.int32, (seg, dm), 0)
    sel_row = lax.broadcasted_iota(jnp.int32, (8, dm), 0)
    picked = jnp.zeros((8, dm), F32)
    gate = jnp.zeros((8, 1), F32)
    routed = []
    for c in range(NUM_ROUTED):
        top = jnp.max(vals, axis=0, keepdims=True)
        pick = jnp.min(jnp.where(vals == top, idxs, n_tok), axis=0, keepdims=True)
        vals = jnp.where(idxs == pick, -jnp.inf, vals)
        tok = jnp.clip(jnp.min(pick), 0, n_tok - 1)
        s = tok // seg
        routed.append((s, tok - s * seg))
        xn = jnp.concatenate([xn_pre[first_rows(s), :], xn_rest[s]], axis=0)
        row = jnp.sum(jnp.where(seg_row == tok - s * seg, xn, 0.0), axis=0, keepdims=True)
        picked = jnp.where(sel_row == c, row, picked)
        gate = jnp.where(sel_row[:, :1] == c, jax.nn.sigmoid(top[:, :1]), gate)
    x_sel[...] = picked
    hidden[...] = jnp.zeros(hidden.shape, F32)
    y_acc[...] = jnp.zeros(y_acc.shape, F32)

    pltpu.make_async_copy(wo_in, wo, sem_wo.at[0]).wait()

    row = lax.broadcasted_iota(jnp.int32, (n_rows, n_rows), 0)
    col = lax.broadcasted_iota(jnp.int32, (n_rows, n_rows), 1)
    visible = (row < n_mem) | (row >= col)
    n_group = n_seg // STEP_UNROLL
    n_chunk = ff // FF_CHUNK
    ffn_start = n_group - n_chunk - 1
    assert ffn_start >= 1

    def ffn_pieces(group):
        def chunk(c):
            return jnp.where((c >= 0) & (c < n_chunk), c, n_chunk)

        up_cols = pl.ds(pl.multiple_of(chunk(group - ffn_start) * FF_CHUNK, FF_CHUNK), FF_CHUNK)
        down_rows = pl.ds(pl.multiple_of(chunk(group - ffn_start - 1) * (FF_CHUNK // 2), FF_CHUNK // 2),
                          FF_CHUNK // 2)
        parts = dm // FF_CHUNK

        def down(n):
            cols = pl.ds(n * FF_CHUNK, FF_CHUNK)
            y_acc[:, cols] += _matmul(hidden[...], _weights(wd[down_rows, cols]))

        def up(i, k):
            w = (wg, wu)[i][pl.ds(k * FF_CHUNK // 2, FF_CHUNK // 2), up_cols]
            r = _matmul(x_sel[:, pl.ds(k * FF_CHUNK, FF_CHUNK)], _weights(w))
            r = r if k == 0 else gate_up[i] + r
            if i == 1 and k == parts - 1:
                g = gate_up[0]
                hidden[...] = g * jax.nn.sigmoid(g) * r
            else:
                gate_up[i] = r

        return ([functools.partial(down, n) for n in range(parts)]
                + [functools.partial(up, i, k) for i in range(2) for k in range(parts)])

    def step(s, memory, fillers):
        rest = xn_rest[s]
        lhs = jnp.concatenate([memory, rest], axis=0).astype(BF16)
        qkv, probs, heads = {}, {}, {}

        def project(j):
            if j == 0:
                acc_first[...] = _matmul(lhs[:, :dm // 2], _weights(wqkv[j, :dm // 4, :]))
                r = acc_first[...] + _matmul(lhs[:, dm // 2:], _weights(wqkv[j, dm // 4:, :]))
            else:
                r = _matmul(lhs, _weights(wqkv[j]))
            qkv[j] = jnp.concatenate([r[:n_mem], pre[j, first_rows(s), :], r[n_mem:]], axis=0)

        def part(j, p, i):
            return qkv[j][:, (3 * p + i) * dh:(3 * p + i + 1) * dh]

        def scores(j):
            for p in range(2):
                sc = _matmul_nt(part(j, p, 0), part(j, p, 1).astype(BF16)) * scale
                sc = jnp.where(visible, sc, MASKED)
                e = jnp.exp(sc - jnp.max(sc, axis=-1, keepdims=True))
                probs[j, p] = (e, jnp.sum(e, axis=-1, keepdims=True))

        def mix(j):
            for p in range(2):
                e, denom = probs[j, p]
                heads[2 * j + p] = _matmul(e, part(j, p, 2).astype(BF16)) / denom

        def out_proj(quarter):
            h0, h1 = quarter * n_pair // 2, (quarter + 1) * n_pair // 2
            o = jnp.concatenate([heads[h] for h in range(h0, h1)], axis=1)
            return _matmul(o, _weights(wo[h0 * dh // 2:h1 * dh // 2, :]))

        for j in range(n_pair):
            project(j)
            if j >= 2:
                mix(j - 2)
            if j >= 1:
                scores(j - 1)
        acc[...] = out_proj(0)
        mix(n_pair - 2)
        scores(n_pair - 1)
        fillers[0]()
        acc[...] += out_proj(1)
        mix(n_pair - 1)
        fillers[1]()
        acc[...] += out_proj(2)
        fillers[2]()
        o = acc[...] + out_proj(3)

        xn = jnp.concatenate([xn_pre[first_rows(s), :], rest], axis=0)
        out_v[s] = ((x_v[s].astype(F32) + o[n_mem:]) + xn).astype(BF16)
        return o[:n_mem]

    def steps(group, carry):
        @pl.when(group == ffn_start)
        def _():
            ffn_copies[0].wait()
            ffn_copies[1].wait()

        @pl.when(group == ffn_start + 1)
        def _():
            ffn_copies[2].wait()

        pieces = ffn_pieces(group)
        assert len(pieces) == 3 * STEP_UNROLL
        memory = mem[...]
        for u in range(STEP_UNROLL):
            memory = step(group * STEP_UNROLL + u, memory, pieces[3 * u:3 * u + 3])
        mem[...] = memory
        for u in range(STEP_UNROLL):
            s = group * STEP_UNROLL + u

            @pl.when((s != routed[0][0]) & (s != routed[1][0]))
            def _():
                out_copy(s).start()

        return carry

    lax.fori_loop(0, n_group, steps, 0)

    y = y_acc[...] * gate
    for c, (s, r) in enumerate(routed):
        upd = jnp.where(seg_row == r, y[c:c + 1], 0.0)
        out_v[s] = (out_v[s].astype(F32) + upd).astype(BF16)

    out_copy(routed[0][0]).start()

    @pl.when(routed[1][0] != routed[0][0])
    def _():
        out_copy(routed[1][0]).start()

    pltpu.make_async_copy(out_v, out_hbm, sem_out.at[0]).wait()


@functools.partial(jax.jit, static_argnames=("A_seg_len",))
def pallas_parallel_sum__memory_aug_recurrent_mem_tr__moe_arch_mod__prompt_kernel(
    A_x: jax.Array,
    A_mem0: jax.Array,
    A_Wq: jax.Array,
    A_Wk: jax.Array,
    A_Wv: jax.Array,
    A_Wo: jax.Array,
    A_seg_len: int,
    B_x: jax.Array,
    B_w_r: jax.Array,
    B_w_gate: jax.Array,
    B_w_up: jax.Array,
    B_w_down: jax.Array,
):
    del B_x
    batch, n_tok, dm = A_x.shape
    _, n_head, dh = A_Wq.shape
    n_mem = A_mem0.shape[1]
    seg = A_seg_len
    n_seg = n_tok // seg
    n_pair = n_head // 2
    ff = B_w_gate.shape[1]
    assert batch == 1 and n_mem == 8 and dh == 128 and seg % 16 == 0 and n_tok == n_seg * seg
    assert n_seg % n_pair == 0 and n_seg % X0_CHUNKS == 0 and n_seg % STEP_UNROLL == 0
    assert (n_pair - 1) % PAIR_UNROLL == 0 and ff % FF_CHUNK == 0

    hbm = pl.BlockSpec(memory_space=pl.ANY)
    vmem = pl.BlockSpec(memory_space=pltpu.VMEM)
    out = pl.pallas_call(
        _kernel,
        out_shape=jax.ShapeDtypeStruct((n_seg, seg, dm), A_x.dtype),
        in_specs=[hbm, vmem, hbm, hbm, hbm, hbm, vmem, hbm, hbm, hbm],
        out_specs=hbm,
        scratch_shapes=[
            pltpu.VMEM((n_seg, seg, dm), BF16),
            pltpu.VMEM((n_seg * PRE, dm), F32),
            pltpu.VMEM((n_seg, seg - PRE, dm), F32),
            pltpu.VMEM((N_STAGE, 3, dm, dh), U32),
            pltpu.VMEM((n_pair, dm // 2, 6 * dh), U32),
            pltpu.VMEM((n_head * dh // 2, dm), U32),
            pltpu.VMEM((n_pair, n_seg * PRE, 6 * dh), F32),
            pltpu.VMEM((n_mem, dm), F32),
            pltpu.VMEM((n_mem + seg, dm), F32),
            pltpu.VMEM((n_mem + seg - PRE, 6 * dh), F32),
            pltpu.VMEM((n_seg, seg, dm), BF16),
            pltpu.VMEM((dm // 2, ff + FF_CHUNK), U32),
            pltpu.VMEM((dm // 2, ff + FF_CHUNK), U32),
            pltpu.VMEM(((ff + FF_CHUNK) // 2, dm), U32),
            pltpu.VMEM((8, dm), F32),
            pltpu.VMEM((2, 8, FF_CHUNK), F32),
            pltpu.VMEM((8, FF_CHUNK), F32),
            pltpu.VMEM((8, dm), F32),
            pltpu.VMEM((NUM_ROUTED, 8, 128), F32),
            pltpu.VMEM((NUM_ROUTED, 8, 128), jnp.int32),
            pltpu.SemaphoreType.DMA((X0_CHUNKS,)),
            pltpu.SemaphoreType.DMA((N_STAGE, 4)),
            pltpu.SemaphoreType.DMA((1,)),
            pltpu.SemaphoreType.DMA((3,)),
            pltpu.SemaphoreType.DMA((1,)),
        ],
        compiler_params=pltpu.CompilerParams(vmem_limit_bytes=120 * 1024 * 1024),
        name="rmt_mod_fused",
    )(
        A_x.reshape(n_seg, seg, dm),
        A_mem0.reshape(n_mem, dm),
        A_Wq,
        A_Wk,
        A_Wv,
        A_Wo.reshape(n_head * dh, dm),
        B_w_r,
        B_w_gate,
        B_w_up,
        B_w_down,
    )
    return out.reshape(batch, n_tok, dm)
```

```python
import functools

import jax
import jax.numpy as jnp
import numpy as np
from jax import lax
from jax.experimental import pallas as pl
from jax.experimental.pallas import tpu as pltpu

F32 = jnp.float32
BF16 = jnp.bfloat16
U32 = jnp.uint32

PRE = 8
LEAD_GROUPS = ((1, 1, 8),)
LOOP_GROUP = (2, 2, 4)
STEP_UNROLL = 4
FF_CHUNK = 256
LN_EPS = 1e-05
MASKED = -1000000000.0
NUM_ROUTED = 2
LOW_HALF = np.uint32(0x0000FFFF)
HIGH_HALF = np.uint32(0xFFFF0000)


def _round_bf16(v):
    return v.astype(BF16).astype(F32)


def _layernorm_rows(x):
    xf = x.astype(F32)
    inv_n = 1.0 / xf.shape[-1]
    mean = jnp.sum(xf, axis=-1, keepdims=True) * inv_n
    cen = xf - mean
    var = jnp.sum(cen * cen, axis=-1, keepdims=True) * inv_n
    eps = jnp.full(var.shape, LN_EPS, BF16).astype(F32)
    std = _round_bf16(jnp.sqrt(_round_bf16(_round_bf16(var) + eps)))
    return _round_bf16(_round_bf16(xf - _round_bf16(mean)) / std)


def _matmul(a, b):
    return lax.dot_general(a, b, (((1,), (0,)), ((), ())), preferred_element_type=F32)


def _matmul_nt(a, b):
    return lax.dot_general(a, b, (((1,), (1,)), ((), ())), preferred_element_type=F32)


def _weights(words):
    return pltpu.bitcast(words, BF16)


def _first_rows(s):
    return pl.ds(pl.multiple_of(s * PRE, PRE), PRE)


def _phase1(x_hbm, mem0_hbm, w_hbm, wo_hbm, wr_hbm,
            x_v, xn_pre, xn_rest, wqkv, wo, pre, mem, best_v, best_i,
            stage, mem0_v, wr_v, wr_rows, sem):
    n_seg, seg, dm = x_v.shape
    n_pair = wqkv.shape[0]
    dh = wqkv.shape[2] // 6
    half_segs = n_seg // 2
    half_rows = half_segs * PRE
    first_loop_pair, loop_pairs, loop_segs = LOOP_GROUP
    n_loop = (n_pair - first_loop_pair) // loop_pairs
    lead_segs = sum(n * per for _, n, per in LEAD_GROUPS)
    assert first_loop_pair + n_loop * loop_pairs == n_pair
    assert lead_segs + n_loop * loop_pairs * loop_segs == n_seg

    w_words = [w.bitcast(U32) for w in w_hbm]

    def x0_copy(c):
        segs = pl.ds(c * half_segs, half_segs)
        return pltpu.make_async_copy(x_hbm.at[segs, pl.ds(0, PRE), :], x_v.at[segs, pl.ds(0, PRE), :],
                                     sem.at[3 * n_pair + c])

    def w_copy(j, i):
        return pltpu.make_async_copy(w_words[i].at[:, j, :], stage.at[j, i], sem.at[3 * j + i])

    def group_copies(g, j0, n, s0, n_s):
        copies = [w_copy(j0 + u, i) for u in range(n) for i in range(3)]
        if n_s:
            segs, rest = pl.ds(s0, n_s), pl.ds(PRE, seg - PRE)
            copies.append(pltpu.make_async_copy(x_hbm.at[segs, rest, :], x_v.at[segs, rest, :],
                                                sem.at[3 * n_pair + 5 + g]))
        return copies

    def loop_copies(t):
        return group_copies(len(LEAD_GROUPS) + t, first_loop_pair + t * loop_pairs, loop_pairs,
                            lead_segs + t * loop_pairs * loop_segs, loop_pairs * loop_segs)

    mem0_copy = pltpu.make_async_copy(mem0_hbm, mem0_v, sem.at[3 * n_pair + 2])
    wr_copy = pltpu.make_async_copy(wr_hbm, wr_v, sem.at[3 * n_pair + 3])
    wo_copy = pltpu.make_async_copy(wo_hbm.bitcast(U32), wo, sem.at[3 * n_pair + 4])

    def split_heads(j, i):
        even = stage[j, i, pl.ds(0, dm // 2, stride=2), :]
        odd = stage[j, i, pl.ds(1, dm // 2, stride=2), :]
        heads = ((even & LOW_HALF) | (odd << 16), (even >> 16) | (odd & HIGH_HALF))
        for p in range(2):
            wqkv[j, :, pl.ds((3 * p + i) * dh, dh)] = heads[p]
        return heads

    def project(j, i, heads, rows=slice(None)):
        for p in range(2):
            pre[j, rows, pl.ds((3 * p + i) * dh, dh)] = _matmul(xn_pre[rows, :], _weights(heads[p]))

    def route_segments(s0, count):
        w_r = wr_rows[...]
        v1, v2, i1, i2 = best_v[0], best_v[1], best_i[0], best_i[1]
        sub = lax.broadcasted_iota(jnp.int32, v1.shape, 0)
        for t in range(count):
            s = s0 + t
            rest = _layernorm_rows(x_v[s, pl.ds(PRE, seg - PRE), :])
            xn_rest[s] = rest
            rows = jnp.concatenate([xn_pre[_first_rows(s), :], rest], axis=0)
            for g in range(seg // 8):
                r = jnp.sum(rows[g * 8:(g + 1) * 8] * w_r, axis=-1, keepdims=True)
                r = jnp.broadcast_to(_round_bf16(r), v1.shape)
                idx = sub + (s * seg + g * 8)
                gt1, gt2 = r > v1, r > v2
                v2 = jnp.where(gt1, v1, jnp.where(gt2, r, v2))
                i2 = jnp.where(gt1, i1, jnp.where(gt2, idx, i2))
                v1 = jnp.where(gt1, r, v1)
                i1 = jnp.where(gt1, idx, i1)
        best_v[0], best_v[1], best_i[0], best_i[1] = v1, v2, i1, i2

    def run_group(j0, n, s0, per_pair):
        for u in range(n):
            for i in range(3):
                project(j0 + u, i, split_heads(j0 + u, i))
            if per_pair:
                route_segments(s0 + u * per_pair, per_pair)

    def norm_half(c):
        rows = x_v[pl.ds(c * half_segs, half_segs), pl.ds(0, PRE), :].astype(F32)
        xn_pre[pl.ds(c * half_rows, half_rows), :] = _layernorm_rows(rows.reshape(half_rows, dm))

    lead, s0 = [], 0
    for g, (j0, n, per_pair) in enumerate(LEAD_GROUPS):
        lead.append((group_copies(g, j0, n, s0, n * per_pair), (j0, n, s0, per_pair)))
        s0 += n * per_pair

    for c in (x0_copy(0), w_copy(0, 0), x0_copy(1), w_copy(0, 1), w_copy(0, 2), mem0_copy, wr_copy):
        c.start()
    for copies, _ in lead:
        for c in copies:
            c.start()
    best_v[...] = jnp.full(best_v.shape, -jnp.inf, F32)
    best_i[...] = jnp.full(best_i.shape, n_seg * seg, jnp.int32)

    x0_copy(0).wait()
    norm_half(0)
    w_copy(0, 0).wait()
    x0_copy(1).wait()
    q_heads = split_heads(0, 0)
    project(0, 0, q_heads, pl.ds(0, half_rows))
    norm_half(1)
    project(0, 0, q_heads, pl.ds(half_rows, half_rows))
    for c in (w_copy(0, 1), w_copy(0, 2), mem0_copy, wr_copy):
        c.wait()
    for c in loop_copies(0):
        c.start()
    for i in (1, 2):
        project(0, i, split_heads(0, i))
    mem[...] = mem0_v[...].astype(F32)
    wr_rows[...] = jnp.broadcast_to(wr_v[...].astype(F32).reshape(1, dm), wr_rows.shape)

    for copies, group in lead:
        for c in copies:
            c.wait()
        run_group(*group)

    def loop_group(t, carry):
        @pl.when(t + 1 < n_loop)
        def _():
            for c in loop_copies(t + 1):
                c.start()

        @pl.when(t + 2 == n_loop)
        def _():
            wo_copy.start()

        for c in loop_copies(t):
            c.wait()
        run_group(first_loop_pair + t * loop_pairs, loop_pairs,
                  lead_segs + t * loop_pairs * loop_segs, loop_segs)
        return carry

    lax.fori_loop(0, n_loop, loop_group, 0)
    wo_copy.wait()


def _phase2(wg_hbm, wu_hbm, wd_hbm, out_hbm,
            x_v, xn_pre, xn_rest, wqkv, wo, pre, mem, best_v, best_i,
            acc, acc_first, out_v, wg, wu, wd, x_sel, gate_up, hidden, y_acc, sem_ffn, sem_out):
    n_seg, seg, dm = x_v.shape
    n_mem = mem.shape[0]
    n_pair = wqkv.shape[0]
    dh = wqkv.shape[2] // 6
    n_rows = n_mem + seg
    n_tok = n_seg * seg
    ff = wd_hbm.shape[0]
    scale = dh ** -0.5

    ffn_copies = [
        pltpu.make_async_copy(wg_hbm.bitcast(U32), wg.at[:, pl.ds(0, ff)], sem_ffn.at[0]),
        pltpu.make_async_copy(wu_hbm.bitcast(U32), wu.at[:, pl.ds(0, ff)], sem_ffn.at[1]),
        pltpu.make_async_copy(wd_hbm.bitcast(U32), wd.at[pl.ds(0, ff // 2), :], sem_ffn.at[2]),
    ]

    def out_copy(s):
        return pltpu.make_async_copy(out_v.at[s], out_hbm.at[s], sem_out.at[0])

    for c in ffn_copies:
        c.start()
    wg[:, pl.ds(ff, FF_CHUNK)] = jnp.zeros((dm // 2, FF_CHUNK), U32)
    wu[:, pl.ds(ff, FF_CHUNK)] = jnp.zeros((dm // 2, FF_CHUNK), U32)
    wd[pl.ds(ff // 2, FF_CHUNK // 2), :] = jnp.zeros((FF_CHUNK // 2, dm), U32)

    vals = jnp.concatenate([best_v[0], best_v[1]], axis=0)
    idxs = jnp.concatenate([best_i[0], best_i[1]], axis=0)
    seg_row = lax.broadcasted_iota(jnp.int32, (seg, dm), 0)
    sel_row = lax.broadcasted_iota(jnp.int32, (8, dm), 0)
    picked = jnp.zeros((8, dm), F32)
    gate = jnp.zeros((8, 1), F32)
    routed = []
    for c in range(NUM_ROUTED):
        top = jnp.max(vals, axis=0, keepdims=True)
        pick = jnp.min(jnp.where(vals == top, idxs, n_tok), axis=0, keepdims=True)
        vals = jnp.where(idxs == pick, -jnp.inf, vals)
        tok = jnp.clip(jnp.min(pick), 0, n_tok - 1)
        s = tok // seg
        routed.append((s, tok - s * seg))
        xn = jnp.concatenate([xn_pre[_first_rows(s), :], xn_rest[s]], axis=0)
        row = jnp.sum(jnp.where(seg_row == tok - s * seg, xn, 0.0), axis=0, keepdims=True)
        picked = jnp.where(sel_row == c, row, picked)
        gate = jnp.where(sel_row[:, :1] == c, jax.nn.sigmoid(top[:, :1]), gate)
    x_sel[...] = picked
    y_acc[...] = jnp.zeros(y_acc.shape, F32)

    row = lax.broadcasted_iota(jnp.int32, (n_rows, n_rows), 0)
    col = lax.broadcasted_iota(jnp.int32, (n_rows, n_rows), 1)
    visible = (row < n_mem) | (row >= col)
    n_group = n_seg // STEP_UNROLL
    n_chunk = ff // FF_CHUNK
    ffn_start = n_group - n_chunk
    assert ffn_start >= 1

    def ffn_pieces(group):
        chunk = jnp.where(group >= ffn_start, group - ffn_start, n_chunk)
        up_cols = pl.ds(pl.multiple_of(chunk * FF_CHUNK, FF_CHUNK), FF_CHUNK)
        down_rows = pl.ds(pl.multiple_of(chunk * (FF_CHUNK // 2), FF_CHUNK // 2), FF_CHUNK // 2)
        parts = dm // FF_CHUNK

        def up(i, k):
            w = (wg, wu)[i][pl.ds(k * FF_CHUNK // 2, FF_CHUNK // 2), up_cols]
            r = _matmul(x_sel[:, pl.ds(k * FF_CHUNK, FF_CHUNK)], _weights(w))
            r = r if k == 0 else gate_up[i] + r
            if i == 1 and k == parts - 1:
                g = gate_up[0]
                hidden[...] = g * jax.nn.sigmoid(g) * r
            else:
                gate_up[i] = r

        def down(n):
            cols = pl.ds(n * FF_CHUNK, FF_CHUNK)
            y_acc[:, cols] += _matmul(hidden[...], _weights(wd[down_rows, cols]))

        return ([functools.partial(up, i, k) for i in range(2) for k in range(parts)]
                + [functools.partial(down, n) for n in range(parts)])

    def step(s, memory, fillers):
        rest = xn_rest[s]
        lhs = jnp.concatenate([memory, rest], axis=0).astype(BF16)
        qkv, probs, heads = {}, {}, {}

        def project(j):
            if j == 0:
                acc_first[...] = _matmul(lhs[:, :dm // 2], _weights(wqkv[j, :dm // 4, :]))
                r = acc_first[...] + _matmul(lhs[:, dm // 2:], _weights(wqkv[j, dm // 4:, :]))
            else:
                r = _matmul(lhs, _weights(wqkv[j]))
            qkv[j] = jnp.concatenate([r[:n_mem], pre[j, _first_rows(s), :], r[n_mem:]], axis=0)

        def part(j, p, i):
            return qkv[j][:, (3 * p + i) * dh:(3 * p + i + 1) * dh]

        def scores(j):
            for p in range(2):
                sc = _matmul_nt(part(j, p, 0), part(j, p, 1).astype(BF16)) * scale
                sc = jnp.where(visible, sc, MASKED)
                e = jnp.exp(sc - jnp.max(sc, axis=-1, keepdims=True))
                probs[j, p] = (e, jnp.sum(e, axis=-1, keepdims=True))

        def mix(j):
            for p in range(2):
                e, denom = probs[j, p]
                heads[2 * j + p] = _matmul(e, part(j, p, 2).astype(BF16)) / denom

        def out_proj(quarter):
            h0, h1 = quarter * n_pair // 2, (quarter + 1) * n_pair // 2
            o = jnp.concatenate([heads[h] for h in range(h0, h1)], axis=1)
            return _matmul(o, _weights(wo[h0 * dh // 2:h1 * dh // 2, :]))

        for j in range(n_pair):
            project(j)
            if j >= 2:
                mix(j - 2)
            if j >= 1:
                scores(j - 1)
        acc[...] = out_proj(0)
        mix(n_pair - 2)
        scores(n_pair - 1)
        fillers[0]()
        acc[...] += out_proj(1)
        mix(n_pair - 1)
        fillers[1]()
        acc[...] += out_proj(2)
        fillers[2]()
        o = acc[...] + out_proj(3)

        xn = jnp.concatenate([xn_pre[_first_rows(s), :], rest], axis=0)
        out_v[s] = ((x_v[s].astype(F32) + o[n_mem:]) + xn).astype(BF16)
        return o[:n_mem]

    def write_group(group, valid):
        for u in range(STEP_UNROLL):
            s = group * STEP_UNROLL + u

            @pl.when(valid & (s != routed[0][0]) & (s != routed[1][0]))
            def _():
                out_copy(s).start()

    def steps(group, carry):
        @pl.when(group == ffn_start)
        def _():
            for c in ffn_copies:
                c.wait()

        pieces = ffn_pieces(group)
        assert len(pieces) == 3 * STEP_UNROLL
        memory = mem[...]
        for u in range(STEP_UNROLL):
            memory = step(group * STEP_UNROLL + u, memory, pieces[3 * u:3 * u + 3])
            if u == 0:
                write_group(jnp.maximum(group - 1, 0), group > 0)
        mem[...] = memory
        return carry

    lax.fori_loop(0, n_group, steps, 0)
    write_group(n_group - 1, True)

    y = y_acc[...] * gate
    for c, (s, r) in enumerate(routed):
        upd = jnp.where(seg_row == r, y[c:c + 1], 0.0)
        out_v[s] = (out_v[s].astype(F32) + upd).astype(BF16)

    out_copy(routed[0][0]).start()

    @pl.when(routed[1][0] != routed[0][0])
    def _():
        out_copy(routed[1][0]).start()

    pltpu.make_async_copy(out_v, out_hbm, sem_out.at[0]).wait()


def _kernel(x_hbm, mem0_hbm, wq_hbm, wk_hbm, wv_hbm, wo_hbm, wr_hbm, wg_hbm, wu_hbm, wd_hbm,
            out_hbm, *shared):
    n_seg, seg, dm = x_hbm.shape
    n_mem = mem0_hbm.shape[0]
    _, n_head, dh = wq_hbm.shape
    n_pair = n_head // 2
    ff = wd_hbm.shape[0]
    dma = pltpu.SemaphoreType.DMA

    pl.run_scoped(
        functools.partial(_phase1, x_hbm, mem0_hbm, (wq_hbm, wk_hbm, wv_hbm), wo_hbm, wr_hbm, *shared),
        pltpu.VMEM((n_pair, 3, dm, dh), U32),
        pltpu.VMEM((n_mem, dm), BF16),
        pltpu.VMEM((dm,), BF16),
        pltpu.VMEM((8, dm), F32),
        dma((4 * n_pair + 5,)),
    )
    pl.run_scoped(
        functools.partial(_phase2, wg_hbm, wu_hbm, wd_hbm, out_hbm, *shared),
        pltpu.VMEM((n_mem + seg, dm), F32),
        pltpu.VMEM((n_mem + seg - PRE, 6 * dh), F32),
        pltpu.VMEM((n_seg, seg, dm), BF16),
        pltpu.VMEM((dm // 2, ff + FF_CHUNK), U32),
        pltpu.VMEM((dm // 2, ff + FF_CHUNK), U32),
        pltpu.VMEM(((ff + FF_CHUNK) // 2, dm), U32),
        pltpu.VMEM((8, dm), F32),
        pltpu.VMEM((2, 8, FF_CHUNK), F32),
        pltpu.VMEM((8, FF_CHUNK), F32),
        pltpu.VMEM((8, dm), F32),
        dma((3,)), dma((1,)),
    )


@functools.partial(jax.jit, static_argnames=("A_seg_len",))
def pallas_parallel_sum__memory_aug_recurrent_mem_tr__moe_arch_mod__prompt_kernel(
    A_x: jax.Array,
    A_mem0: jax.Array,
    A_Wq: jax.Array,
    A_Wk: jax.Array,
    A_Wv: jax.Array,
    A_Wo: jax.Array,
    A_seg_len: int,
    B_x: jax.Array,
    B_w_r: jax.Array,
    B_w_gate: jax.Array,
    B_w_up: jax.Array,
    B_w_down: jax.Array,
):
    del B_x
    batch, n_tok, dm = A_x.shape
    _, n_head, dh = A_Wq.shape
    n_mem = A_mem0.shape[1]
    seg = A_seg_len
    n_seg = n_tok // seg
    n_pair = n_head // 2
    ff = B_w_gate.shape[1]
    assert batch == 1 and n_mem == 8 and dh == 128 and seg % 16 == 0 and n_tok == n_seg * seg
    assert n_seg % 2 == 0 and n_seg % STEP_UNROLL == 0 and ff % FF_CHUNK == 0

    hbm = pl.BlockSpec(memory_space=pl.ANY)
    out = pl.pallas_call(
        _kernel,
        out_shape=jax.ShapeDtypeStruct((n_seg, seg, dm), A_x.dtype),
        in_specs=[hbm] * 10,
        out_specs=hbm,
        scratch_shapes=[
            pltpu.VMEM((n_seg, seg, dm), BF16),
            pltpu.VMEM((n_seg * PRE, dm), F32),
            pltpu.VMEM((n_seg, seg - PRE, dm), F32),
            pltpu.VMEM((n_pair, dm // 2, 6 * dh), U32),
            pltpu.VMEM((n_head * dh // 2, dm), U32),
            pltpu.VMEM((n_pair, n_seg * PRE, 6 * dh), F32),
            pltpu.VMEM((n_mem, dm), F32),
            pltpu.VMEM((NUM_ROUTED, 8, 128), F32),
            pltpu.VMEM((NUM_ROUTED, 8, 128), jnp.int32),
        ],
        compiler_params=pltpu.CompilerParams(
            vmem_limit_bytes=120 * 1024 * 1024,
            flags={"XLA_TPU_EVENLY_DISTRIBUTE_CRITICAL_NODES": True},
        ),
        name="rmt_mod_fused",
    )(
        A_x.reshape(n_seg, seg, dm),
        A_mem0.reshape(n_mem, dm),
        A_Wq,
        A_Wk,
        A_Wv,
        A_Wo.reshape(n_head * dh, dm),
        B_w_r,
        B_w_gate,
        B_w_up,
        B_w_down,
    )
    return out.reshape(batch, n_tok, dm)
```

```python
import functools

import jax
import jax.numpy as jnp
import numpy as np
from jax import lax
from jax.experimental import pallas as pl
from jax.experimental.pallas import tpu as pltpu

F32 = jnp.float32
BF16 = jnp.bfloat16
U32 = jnp.uint32

PRE = 8
PAIR_GROUP = 2
WO_PIECES = 4
STEP_UNROLL = 4
FF_CHUNK = 256
LN_EPS = 1e-05
MASKED = -1000000000.0
NUM_ROUTED = 2
LOW_HALF = np.uint32(0x0000FFFF)
HIGH_HALF = np.uint32(0xFFFF0000)


def _round_bf16(v):
    return v.astype(BF16).astype(F32)


def _layernorm_rows(x):
    xf = x.astype(F32)
    inv_n = 1.0 / xf.shape[-1]
    mean = jnp.sum(xf, axis=-1, keepdims=True) * inv_n
    cen = xf - mean
    var = jnp.sum(cen * cen, axis=-1, keepdims=True) * inv_n
    eps = jnp.full(var.shape, LN_EPS, BF16).astype(F32)
    std = _round_bf16(jnp.sqrt(_round_bf16(_round_bf16(var) + eps)))
    return _round_bf16(_round_bf16(xf - _round_bf16(mean)) / std)


def _matmul(a, b):
    return lax.dot_general(a, b, (((1,), (0,)), ((), ())), preferred_element_type=F32)


def _matmul_nt(a, b):
    return lax.dot_general(a, b, (((1,), (1,)), ((), ())), preferred_element_type=F32)


def _weights(words):
    return pltpu.bitcast(words, BF16)


def _first_rows(s):
    return pl.ds(pl.multiple_of(s * PRE, PRE), PRE)


def _kernel(x_hbm, mem0_hbm, wq_hbm, wk_hbm, wv_hbm, wo_hbm, wr_hbm, wg_hbm, wu_hbm, wd_hbm,
            out_hbm,
            x_v, xn_pre, xn_rest, stage, wqkv, wo, pre, mem0_v, mem, acc, acc_first, out_v,
            wr_v, wr_rows, best_v, best_i, wg, wu, wd, x_sel, gate, gate_up, hidden, y_acc,
            sem_in, sem_ffn, sem_out):
    n_seg, seg, dm = x_v.shape
    n_mem = mem.shape[0]
    n_pair = wqkv.shape[0]
    dh = wqkv.shape[2] // 6
    n_rows = n_mem + seg
    n_tok = n_seg * seg
    ff = wd_hbm.shape[0]
    seg_row = lax.broadcasted_iota(jnp.int32, (seg, dm), 0)

    def normalised(s):
        return jnp.concatenate([xn_pre[_first_rows(s), :], xn_rest[s]], axis=0)

    n_slot = stage.shape[0]
    n_load = n_pair // PAIR_GROUP
    group_segs = n_seg // n_load
    half_segs = n_seg // 2
    half_rows = half_segs * PRE

    w_words = [w.bitcast(U32) for w in (wq_hbm, wk_hbm, wv_hbm)]
    wo_words = wo_hbm.bitcast(U32)

    def w_copy(j, i):
        slot = j % n_slot
        return pltpu.make_async_copy(w_words[i].at[:, j, :], stage.at[slot, i], sem_in.at[3 * slot + i])

    def x0_copy(c):
        segs = pl.ds(c * half_segs, half_segs)
        return pltpu.make_async_copy(x_hbm.at[segs, pl.ds(0, PRE), :], x_v.at[segs, pl.ds(0, PRE), :],
                                     sem_in.at[3 * n_slot + c])

    def x_copy(t):
        segs, rest = pl.ds(t * group_segs, group_segs), pl.ds(PRE, seg - PRE)
        return pltpu.make_async_copy(x_hbm.at[segs, rest, :], x_v.at[segs, rest, :],
                                     sem_in.at[3 * n_slot + 2 + t % 2])

    def group_copies(t, first=0):
        return ([w_copy(t * PAIR_GROUP + u, i) for u in range(first, PAIR_GROUP) for i in range(3)]
                + [x_copy(t)])

    def wo_copy(piece):
        rows = pl.ds(piece * (wo.shape[0] // WO_PIECES), wo.shape[0] // WO_PIECES)
        return pltpu.make_async_copy(wo_words.at[rows, :], wo.at[rows, :], sem_in.at[3 * n_slot + 4])

    mem0_copy = pltpu.make_async_copy(mem0_hbm, mem0_v, sem_in.at[3 * n_slot + 5])
    wr_copy = pltpu.make_async_copy(wr_hbm, wr_v, sem_in.at[3 * n_slot + 6])

    def split_heads(j, i):
        even = stage[j % n_slot, i, pl.ds(0, dm // 2, stride=2), :]
        odd = stage[j % n_slot, i, pl.ds(1, dm // 2, stride=2), :]
        heads = ((even & LOW_HALF) | (odd << 16), (even >> 16) | (odd & HIGH_HALF))
        for p in range(2):
            wqkv[j, :, pl.ds((3 * p + i) * dh, dh)] = heads[p]
        return heads

    def project_first_rows(j, i, heads, rows=slice(None)):
        for p in range(2):
            pre[j, rows, pl.ds((3 * p + i) * dh, dh)] = _matmul(xn_pre[rows, :], _weights(heads[p]))

    def score_segments(s0, count):
        v1, v2, i1, i2 = best_v[0], best_v[1], best_i[0], best_i[1]
        sub = lax.broadcasted_iota(jnp.int32, v1.shape, 0)
        for t in range(count):
            s = s0 + t
            rest = _layernorm_rows(x_v[s, pl.ds(PRE, seg - PRE), :])
            xn_rest[s] = rest
            rows = jnp.concatenate([xn_pre[_first_rows(s), :], rest], axis=0)
            for g in range(seg // 8):
                r = jnp.sum(rows[g * 8:(g + 1) * 8] * wr_rows[...], axis=-1, keepdims=True)
                r = jnp.broadcast_to(_round_bf16(r), v1.shape)
                idx = sub + (s * seg + g * 8)
                gt1, gt2 = r > v1, r > v2
                v2 = jnp.where(gt1, v1, jnp.where(gt2, r, v2))
                i2 = jnp.where(gt1, i1, jnp.where(gt2, idx, i2))
                v1 = jnp.where(gt1, r, v1)
                i1 = jnp.where(gt1, idx, i1)
        best_v[0], best_v[1], best_i[0], best_i[1] = v1, v2, i1, i2

    def norm_half(c):
        rows = x_v[pl.ds(c * half_segs, half_segs), pl.ds(0, PRE), :].astype(F32)
        xn_pre[pl.ds(c * half_rows, half_rows), :] = _layernorm_rows(rows.reshape(half_rows, dm))

    for c in ([x0_copy(0), w_copy(0, 0), x0_copy(1), w_copy(0, 1), w_copy(0, 2), mem0_copy, wr_copy]
              + group_copies(0, first=1) + group_copies(1)):
        c.start()
    best_v[...] = jnp.full(best_v.shape, -jnp.inf, F32)
    best_i[...] = jnp.full(best_i.shape, n_tok, jnp.int32)
    y_acc[...] = jnp.zeros(y_acc.shape, F32)
    wg[:, pl.ds(ff, FF_CHUNK)] = jnp.zeros((dm // 2, FF_CHUNK), U32)
    wu[:, pl.ds(ff, FF_CHUNK)] = jnp.zeros((dm // 2, FF_CHUNK), U32)
    wd[pl.ds(ff // 2, FF_CHUNK // 2), :] = jnp.zeros((FF_CHUNK // 2, dm), U32)

    x0_copy(0).wait()
    norm_half(0)
    w_copy(0, 0).wait()
    x0_copy(1).wait()
    q_heads = split_heads(0, 0)
    project_first_rows(0, 0, q_heads, pl.ds(0, half_rows))
    norm_half(1)
    project_first_rows(0, 0, q_heads, pl.ds(half_rows, half_rows))
    for c in (w_copy(0, 1), w_copy(0, 2), mem0_copy, wr_copy):
        c.wait()
    for i in (1, 2):
        project_first_rows(0, i, split_heads(0, i))
    mem[...] = mem0_v[...].astype(F32)
    wr_rows[...] = jnp.broadcast_to(wr_v[...].astype(F32).reshape(1, dm), wr_rows.shape)

    for c in group_copies(0, first=1):
        c.wait()
    for j in range(1, PAIR_GROUP):
        for i in range(3):
            project_first_rows(j, i, split_heads(j, i))
    score_segments(0, group_segs)

    def load_group(t, carry):
        for c in group_copies(t):
            c.wait()
        for c in group_copies(jnp.minimum(t + 1, n_load - 1)):
            pl.when(t + 1 < n_load)(c.start)
        pl.when(t <= WO_PIECES)(wo_copy(jnp.minimum(t, WO_PIECES) - 1).start)
        for u in range(PAIR_GROUP):
            j = t * PAIR_GROUP + u
            for i in range(3):
                project_first_rows(j, i, split_heads(j, i))
            score_segments(t * group_segs + u * (group_segs // PAIR_GROUP), group_segs // PAIR_GROUP)
        return carry

    lax.fori_loop(1, n_load, load_group, 0)

    ffn_copies = [
        pltpu.make_async_copy(wg_hbm.bitcast(U32), wg.at[:, pl.ds(0, ff)], sem_ffn.at[0]),
        pltpu.make_async_copy(wu_hbm.bitcast(U32), wu.at[:, pl.ds(0, ff)], sem_ffn.at[1]),
        pltpu.make_async_copy(wd_hbm.bitcast(U32), wd.at[pl.ds(0, ff // 2), :], sem_ffn.at[2]),
    ]
    for c in ffn_copies:
        c.start()

    vals = jnp.concatenate([best_v[0], best_v[1]], axis=0)
    idxs = jnp.concatenate([best_i[0], best_i[1]], axis=0)
    sel_row = lax.broadcasted_iota(jnp.int32, x_sel.shape, 0)
    picked = jnp.zeros(x_sel.shape, F32)
    weight = jnp.zeros(gate.shape, F32)
    routed = []
    for c in range(NUM_ROUTED):
        top = jnp.max(vals, axis=0, keepdims=True)
        pick = jnp.min(jnp.where(vals == top, idxs, n_tok), axis=0, keepdims=True)
        vals = jnp.where(idxs == pick, -jnp.inf, vals)
        tok = jnp.clip(jnp.min(pick), 0, n_tok - 1)
        s = tok // seg
        routed.append((s, tok - s * seg))
        row = jnp.sum(jnp.where(seg_row == tok - s * seg, normalised(s), 0.0), axis=0, keepdims=True)
        picked = jnp.where(sel_row == c, row, picked)
        weight = jnp.where(sel_row[:, :gate.shape[1]] == c, jax.nn.sigmoid(top), weight)
    x_sel[...] = picked
    gate[...] = weight

    pltpu.make_async_copy(wo_words, wo, sem_in.at[3 * n_slot + 4]).wait()

    scale = dh ** -0.5
    row = lax.broadcasted_iota(jnp.int32, (n_rows, n_rows), 0)
    col = lax.broadcasted_iota(jnp.int32, (n_rows, n_rows), 1)
    visible = (row < n_mem) | (row >= col)
    n_group = n_seg // STEP_UNROLL
    n_chunk = ff // FF_CHUNK
    ffn_start = n_group - n_chunk
    assert ffn_start >= 1

    def out_copy(s):
        return pltpu.make_async_copy(out_v.at[s], out_hbm.at[s], sem_out.at[0])

    def ffn_pieces(group):
        chunk = jnp.where(group >= ffn_start, group - ffn_start, n_chunk)
        up_cols = pl.ds(pl.multiple_of(chunk * FF_CHUNK, FF_CHUNK), FF_CHUNK)
        down_rows = pl.ds(pl.multiple_of(chunk * (FF_CHUNK // 2), FF_CHUNK // 2), FF_CHUNK // 2)
        parts = dm // FF_CHUNK

        def up(i, k):
            w = (wg, wu)[i][pl.ds(k * FF_CHUNK // 2, FF_CHUNK // 2), up_cols]
            r = _matmul(x_sel[:, pl.ds(k * FF_CHUNK, FF_CHUNK)], _weights(w))
            r = r if k == 0 else gate_up[i] + r
            if i == 1 and k == parts - 1:
                g = gate_up[0]
                hidden[...] = g * jax.nn.sigmoid(g) * r
            else:
                gate_up[i] = r

        def down(n):
            cols = pl.ds(n * FF_CHUNK, FF_CHUNK)
            y_acc[:, cols] += _matmul(hidden[...], _weights(wd[down_rows, cols]))

        return ([functools.partial(up, i, k) for i in range(2) for k in range(parts)]
                + [functools.partial(down, n) for n in range(parts)])

    def step(s, memory, fillers):
        lhs = jnp.concatenate([memory, xn_rest[s]], axis=0).astype(BF16)
        qkv, probs, heads = {}, {}, {}

        def project(j):
            if j == 0:
                acc_first[...] = _matmul(lhs[:, :dm // 2], _weights(wqkv[j, :dm // 4, :]))
                r = acc_first[...] + _matmul(lhs[:, dm // 2:], _weights(wqkv[j, dm // 4:, :]))
            else:
                r = _matmul(lhs, _weights(wqkv[j]))
            qkv[j] = jnp.concatenate([r[:n_mem], pre[j, _first_rows(s), :], r[n_mem:]], axis=0)

        def part(j, p, i):
            return qkv[j][:, (3 * p + i) * dh:(3 * p + i + 1) * dh]

        def scores(j):
            for p in range(2):
                sc = _matmul_nt(part(j, p, 0), part(j, p, 1).astype(BF16)) * scale
                sc = jnp.where(visible, sc, MASKED)
                e = jnp.exp(sc - jnp.max(sc, axis=-1, keepdims=True))
                probs[j, p] = (e, jnp.sum(e, axis=-1, keepdims=True))

        def mix(j):
            for p in range(2):
                e, denom = probs[j, p]
                heads[2 * j + p] = _matmul(e, part(j, p, 2).astype(BF16)) / denom

        def out_proj(quarter):
            h0, h1 = quarter * n_pair // 2, (quarter + 1) * n_pair // 2
            o = jnp.concatenate([heads[h] for h in range(h0, h1)], axis=1)
            return _matmul(o, _weights(wo[h0 * dh // 2:h1 * dh // 2, :]))

        for j in range(n_pair):
            project(j)
            if j >= 2:
                mix(j - 2)
            if j >= 1:
                scores(j - 1)
        acc[...] = out_proj(0)
        mix(n_pair - 2)
        scores(n_pair - 1)
        fillers[0]()
        acc[...] += out_proj(1)
        mix(n_pair - 1)
        fillers[1]()
        acc[...] += out_proj(2)
        fillers[2]()
        o = acc[...] + out_proj(3)

        out_v[s] = ((x_v[s].astype(F32) + o[n_mem:]) + normalised(s)).astype(BF16)
        return o[:n_mem]

    def write_group(group, valid):
        for u in range(STEP_UNROLL):
            s = group * STEP_UNROLL + u
            pl.when(valid & (s != routed[0][0]) & (s != routed[1][0]))(out_copy(s).start)

    def steps(group, carry):
        @pl.when(group == ffn_start)
        def _():
            for c in ffn_copies:
                c.wait()

        pieces = ffn_pieces(group)
        assert len(pieces) == 3 * STEP_UNROLL
        memory = mem[...]
        for u in range(STEP_UNROLL):
            memory = step(group * STEP_UNROLL + u, memory, pieces[3 * u:3 * u + 3])
            if u == 0:
                write_group(jnp.maximum(group - 1, 0), group > 0)
        mem[...] = memory
        return carry

    lax.fori_loop(0, n_group, steps, 0)
    write_group(n_group - 1, True)

    y = y_acc[...] * gate[:, :1]
    for c, (s, r) in enumerate(routed):
        upd = jnp.where(seg_row == r, y[c:c + 1], 0.0)
        out_v[s] = (out_v[s].astype(F32) + upd).astype(BF16)
    out_copy(routed[0][0]).start()
    pl.when(routed[1][0] != routed[0][0])(out_copy(routed[1][0]).start)
    pltpu.make_async_copy(out_v, out_hbm, sem_out.at[0]).wait()


@functools.partial(jax.jit, static_argnames=("A_seg_len",))
def pallas_parallel_sum__memory_aug_recurrent_mem_tr__moe_arch_mod__prompt_kernel(
    A_x: jax.Array,
    A_mem0: jax.Array,
    A_Wq: jax.Array,
    A_Wk: jax.Array,
    A_Wv: jax.Array,
    A_Wo: jax.Array,
    A_seg_len: int,
    B_x: jax.Array,
    B_w_r: jax.Array,
    B_w_gate: jax.Array,
    B_w_up: jax.Array,
    B_w_down: jax.Array,
):
    del B_x
    batch, n_tok, dm = A_x.shape
    _, n_head, dh = A_Wq.shape
    n_mem = A_mem0.shape[1]
    seg = A_seg_len
    n_seg = n_tok // seg
    n_pair = n_head // 2
    n_slot = 2 * PAIR_GROUP
    ff = B_w_gate.shape[1]
    assert batch == 1 and n_mem == 8 and dh == 128 and seg % 16 == 0 and n_tok == n_seg * seg
    assert n_pair % PAIR_GROUP == 0 and n_seg % n_pair == 0 and n_pair // PAIR_GROUP > WO_PIECES
    assert n_seg % STEP_UNROLL == 0 and ff % FF_CHUNK == 0

    hbm = pl.BlockSpec(memory_space=pl.ANY)
    out = pl.pallas_call(
        _kernel,
        out_shape=jax.ShapeDtypeStruct((n_seg, seg, dm), A_x.dtype),
        in_specs=[hbm] * 10,
        out_specs=hbm,
        scratch_shapes=[
            pltpu.VMEM((n_seg, seg, dm), BF16),
            pltpu.VMEM((n_seg * PRE, dm), F32),
            pltpu.VMEM((n_seg, seg - PRE, dm), F32),
            pltpu.VMEM((n_slot, 3, dm, dh), U32),
            pltpu.VMEM((n_pair, dm // 2, 6 * dh), U32),
            pltpu.VMEM((n_head * dh // 2, dm), U32),
            pltpu.VMEM((n_pair, n_seg * PRE, 6 * dh), F32),
            pltpu.VMEM((n_mem, dm), BF16),
            pltpu.VMEM((n_mem, dm), F32),
            pltpu.VMEM((n_mem + seg, dm), F32),
            pltpu.VMEM((n_mem + seg - PRE, 6 * dh), F32),
            pltpu.VMEM((n_seg, seg, dm), BF16),
            pltpu.VMEM((dm,), BF16),
            pltpu.VMEM((8, dm), F32),
            pltpu.VMEM((NUM_ROUTED, 8, 128), F32),
            pltpu.VMEM((NUM_ROUTED, 8, 128), jnp.int32),
            pltpu.VMEM((dm // 2, ff + FF_CHUNK), U32),
            pltpu.VMEM((dm // 2, ff + FF_CHUNK), U32),
            pltpu.VMEM(((ff + FF_CHUNK) // 2, dm), U32),
            pltpu.VMEM((8, dm), F32),
            pltpu.VMEM((8, 128), F32),
            pltpu.VMEM((2, 8, FF_CHUNK), F32),
            pltpu.VMEM((8, FF_CHUNK), F32),
            pltpu.VMEM((8, dm), F32),
            pltpu.SemaphoreType.DMA((3 * n_slot + 7,)),
            pltpu.SemaphoreType.DMA((3,)),
            pltpu.SemaphoreType.DMA((1,)),
        ],
        compiler_params=pltpu.CompilerParams(
            vmem_limit_bytes=120 * 1024 * 1024,
            flags={"XLA_TPU_EVENLY_DISTRIBUTE_CRITICAL_NODES": True},
        ),
        name="rmt_mod_fused",
    )(
        A_x.reshape(n_seg, seg, dm),
        A_mem0.reshape(n_mem, dm),
        A_Wq,
        A_Wk,
        A_Wv,
        A_Wo.reshape(n_head * dh, dm),
        B_w_r,
        B_w_gate,
        B_w_up,
        B_w_down,
    )
    return out.reshape(batch, n_tok, dm)
```

```python
import functools

import jax
import jax.numpy as jnp
import numpy as np
from jax import lax
from jax.experimental import pallas as pl
from jax.experimental.pallas import tpu as pltpu

F32 = jnp.float32
BF16 = jnp.bfloat16
U32 = jnp.uint32

PRE = 8
PAIR_GROUP = 2
STEP_UNROLL = 4
FF_CHUNK = 256
LN_EPS = 1e-05
MASKED = -1000000000.0
NUM_ROUTED = 2
LOW_HALF = np.uint32(0x0000FFFF)
HIGH_HALF = np.uint32(0xFFFF0000)


def _round_bf16(v):
    return v.astype(BF16).astype(F32)


def _layernorm_rows(x):
    xf = x.astype(F32)
    inv_n = 1.0 / xf.shape[-1]
    mean = jnp.sum(xf, axis=-1, keepdims=True) * inv_n
    cen = xf - mean
    var = jnp.sum(cen * cen, axis=-1, keepdims=True) * inv_n
    eps = jnp.full(var.shape, LN_EPS, BF16).astype(F32)
    std = _round_bf16(jnp.sqrt(_round_bf16(_round_bf16(var) + eps)))
    return _round_bf16(_round_bf16(xf - _round_bf16(mean)) / std)


def _matmul(a, b):
    return lax.dot_general(a, b, (((1,), (0,)), ((), ())), preferred_element_type=F32)


def _matmul_nt(a, b):
    return lax.dot_general(a, b, (((1,), (1,)), ((), ())), preferred_element_type=F32)


def _weights(words):
    return pltpu.bitcast(words, BF16)


def _first_rows(s):
    return pl.ds(pl.multiple_of(s * PRE, PRE), PRE)


def _kernel(x_hbm, mem0_hbm, wq_hbm, wk_hbm, wv_hbm, wo_hbm, wr_hbm, wg_hbm, wu_hbm, wd_hbm,
            out_hbm,
            x_v, xn_pre, xn_rest, stage, wqkv, wo, pre, mem, acc, acc_first, out_v, wr_rows, wg,
            wu, wd, x_sel, y_acc, mem0_v, gate_up, hidden, best_v, best_i, gate, wr_v,
            sem_w, sem_out):
    n_seg, seg, dm = x_v.shape
    n_mem = mem.shape[0]
    n_pair = wqkv.shape[0]
    dh = wqkv.shape[2] // 6
    n_rows = n_mem + seg
    n_tok = n_seg * seg
    ff = wd_hbm.shape[0]
    seg_row = lax.broadcasted_iota(jnp.int32, (seg, dm), 0)

    def normalised(s):
        return jnp.concatenate([xn_pre[_first_rows(s), :], xn_rest[s]], axis=0)

    n_load = n_pair // PAIR_GROUP
    group_segs = n_seg // n_load
    half_segs = n_seg // 2
    half_rows = half_segs * PRE

    w_words = [w.bitcast(U32) for w in (wq_hbm, wk_hbm, wv_hbm)]

    def w_copy(j, i):
        return pltpu.make_async_copy(w_words[i].at[:, j, :], stage.at[j, i], sem_w.at[3 * j + i])

    def x0_copy(c):
        segs = pl.ds(c * half_segs, half_segs)
        return pltpu.make_async_copy(x_hbm.at[segs, pl.ds(0, PRE), :], x_v.at[segs, pl.ds(0, PRE), :],
                                     sem_w.at[3 * n_pair + c])

    def x_copy(t):
        segs, rest = pl.ds(t * group_segs, group_segs), pl.ds(PRE, seg - PRE)
        return pltpu.make_async_copy(x_hbm.at[segs, rest, :], x_v.at[segs, rest, :],
                                     sem_w.at[3 * n_pair + 8 + t])

    def group_copies(t, first=0):
        return ([w_copy(t * PAIR_GROUP + u, i) for u in range(first, PAIR_GROUP) for i in range(3)]
                + [x_copy(t)])

    mem0_copy, wr_copy, wo_copy, *ffn_copies = (
        pltpu.make_async_copy(src, dst, sem_w.at[3 * n_pair + 2 + i]) for i, (src, dst) in enumerate((
            (mem0_hbm, mem0_v),
            (wr_hbm, wr_v),
            (wo_hbm.bitcast(U32), wo),
            (wg_hbm.bitcast(U32), wg.at[:, pl.ds(0, ff)]),
            (wu_hbm.bitcast(U32), wu.at[:, pl.ds(0, ff)]),
            (wd_hbm.bitcast(U32), wd.at[pl.ds(0, ff // 2), :]))))

    def split_heads(j, i):
        even = stage[j, i, pl.ds(0, dm // 2, stride=2), :]
        odd = stage[j, i, pl.ds(1, dm // 2, stride=2), :]
        heads = ((even & LOW_HALF) | (odd << 16), (even >> 16) | (odd & HIGH_HALF))
        for p in range(2):
            wqkv[j, :, pl.ds((3 * p + i) * dh, dh)] = heads[p]
        return heads

    def project_first_rows(j, i, heads, rows=slice(None)):
        for p in range(2):
            pre[j, rows, pl.ds((3 * p + i) * dh, dh)] = _matmul(xn_pre[rows, :], _weights(heads[p]))

    def score_segments(s0, count):
        v1, v2, i1, i2 = best_v[0], best_v[1], best_i[0], best_i[1]
        sub = lax.broadcasted_iota(jnp.int32, v1.shape, 0)
        for t in range(count):
            s = s0 + t
            rest = _layernorm_rows(x_v[s, pl.ds(PRE, seg - PRE), :])
            xn_rest[s] = rest
            rows = jnp.concatenate([xn_pre[_first_rows(s), :], rest], axis=0)
            for g in range(seg // 8):
                r = jnp.sum(rows[g * 8:(g + 1) * 8] * wr_rows[...], axis=-1, keepdims=True)
                r = jnp.broadcast_to(_round_bf16(r), v1.shape)
                idx = sub + (s * seg + g * 8)
                gt1, gt2 = r > v1, r > v2
                v2 = jnp.where(gt1, v1, jnp.where(gt2, r, v2))
                i2 = jnp.where(gt1, i1, jnp.where(gt2, idx, i2))
                v1 = jnp.where(gt1, r, v1)
                i1 = jnp.where(gt1, idx, i1)
        best_v[0], best_v[1], best_i[0], best_i[1] = v1, v2, i1, i2

    def norm_half(c):
        rows = x_v[pl.ds(c * half_segs, half_segs), pl.ds(0, PRE), :].astype(F32)
        xn_pre[pl.ds(c * half_rows, half_rows), :] = _layernorm_rows(rows.reshape(half_rows, dm))

    for c in ([x0_copy(0), w_copy(0, 0), x0_copy(1), w_copy(0, 1), w_copy(0, 2), mem0_copy, wr_copy]
              + group_copies(0, first=1) + [c for t in range(1, n_load) for c in group_copies(t)]
              + [wo_copy] + ffn_copies):
        c.start()
    best_v[...] = jnp.full(best_v.shape, -jnp.inf, F32)
    best_i[...] = jnp.full(best_i.shape, n_tok, jnp.int32)
    y_acc[...] = jnp.zeros(y_acc.shape, F32)
    wg[:, pl.ds(ff, FF_CHUNK)] = jnp.zeros((dm // 2, FF_CHUNK), U32)
    wu[:, pl.ds(ff, FF_CHUNK)] = jnp.zeros((dm // 2, FF_CHUNK), U32)
    wd[pl.ds(ff // 2, FF_CHUNK // 2), :] = jnp.zeros((FF_CHUNK // 2, dm), U32)

    x0_copy(0).wait()
    norm_half(0)
    w_copy(0, 0).wait()
    x0_copy(1).wait()
    q_heads = split_heads(0, 0)
    project_first_rows(0, 0, q_heads, pl.ds(0, half_rows))
    norm_half(1)
    project_first_rows(0, 0, q_heads, pl.ds(half_rows, half_rows))
    for c in (w_copy(0, 1), w_copy(0, 2), mem0_copy, wr_copy):
        c.wait()
    for i in (1, 2):
        project_first_rows(0, i, split_heads(0, i))
    mem[...] = mem0_v[...].astype(F32)
    wr_rows[...] = jnp.broadcast_to(wr_v[...].astype(F32).reshape(1, dm), wr_rows.shape)

    def load_group(t, carry, first=0):
        for c in group_copies(t, first):
            c.wait()
        segs = group_segs // (PAIR_GROUP - first)
        for u in range(first, PAIR_GROUP):
            j = t * PAIR_GROUP + u
            for i in range(3):
                project_first_rows(j, i, split_heads(j, i))
            score_segments(t * group_segs + (u - first) * segs, segs)
        return carry

    load_group(0, 0, first=1)
    lax.fori_loop(1, n_load, load_group, 0)

    vals = jnp.concatenate([best_v[0], best_v[1]], axis=0)
    idxs = jnp.concatenate([best_i[0], best_i[1]], axis=0)
    sel_row = lax.broadcasted_iota(jnp.int32, x_sel.shape, 0)
    picked = jnp.zeros(x_sel.shape, F32)
    weight = jnp.zeros(gate.shape, F32)
    routed = []
    for c in range(NUM_ROUTED):
        top = jnp.max(vals, axis=0, keepdims=True)
        pick = jnp.min(jnp.where(vals == top, idxs, n_tok), axis=0, keepdims=True)
        vals = jnp.where(idxs == pick, -jnp.inf, vals)
        tok = jnp.clip(jnp.min(pick), 0, n_tok - 1)
        s = tok // seg
        routed.append((s, tok - s * seg))
        row = jnp.sum(jnp.where(seg_row == tok - s * seg, normalised(s), 0.0), axis=0, keepdims=True)
        picked = jnp.where(sel_row == c, row, picked)
        weight = jnp.where(sel_row[:, :gate.shape[1]] == c, jax.nn.sigmoid(top), weight)
    x_sel[...] = picked
    gate[...] = weight

    wo_copy.wait()

    scale = dh ** -0.5
    row = lax.broadcasted_iota(jnp.int32, (n_rows, n_rows), 0)
    col = lax.broadcasted_iota(jnp.int32, (n_rows, n_rows), 1)
    visible = (row < n_mem) | (row >= col)
    n_group = n_seg // STEP_UNROLL
    n_chunk = ff // FF_CHUNK
    ffn_start = n_group - n_chunk
    assert ffn_start >= 1

    def out_copy(s):
        return pltpu.make_async_copy(out_v.at[s], out_hbm.at[s], sem_out.at[0])

    def ffn_pieces(group):
        chunk = jnp.where(group >= ffn_start, group - ffn_start, n_chunk)
        up_cols = pl.ds(pl.multiple_of(chunk * FF_CHUNK, FF_CHUNK), FF_CHUNK)
        down_rows = pl.ds(pl.multiple_of(chunk * (FF_CHUNK // 2), FF_CHUNK // 2), FF_CHUNK // 2)
        parts = dm // FF_CHUNK

        def up(i, k):
            w = (wg, wu)[i][pl.ds(k * FF_CHUNK // 2, FF_CHUNK // 2), up_cols]
            r = _matmul(x_sel[:, pl.ds(k * FF_CHUNK, FF_CHUNK)], _weights(w))
            r = r if k == 0 else gate_up[i] + r
            if i == 1 and k == parts - 1:
                g = gate_up[0]
                hidden[...] = g * jax.nn.sigmoid(g) * r
            else:
                gate_up[i] = r

        def down(n):
            cols = pl.ds(n * FF_CHUNK, FF_CHUNK)
            y_acc[:, cols] += _matmul(hidden[...], _weights(wd[down_rows, cols]))

        return ([functools.partial(up, i, k) for i in range(2) for k in range(parts)]
                + [functools.partial(down, n) for n in range(parts)])

    def step(s, memory, fillers):
        lhs = jnp.concatenate([memory, xn_rest[s]], axis=0).astype(BF16)
        qkv, probs, heads = {}, {}, {}

        def project(j):
            if j == 0:
                acc_first[...] = _matmul(lhs[:, :dm // 2], _weights(wqkv[j, :dm // 4, :]))
                r = acc_first[...] + _matmul(lhs[:, dm // 2:], _weights(wqkv[j, dm // 4:, :]))
            else:
                r = _matmul(lhs, _weights(wqkv[j]))
            qkv[j] = jnp.concatenate([r[:n_mem], pre[j, _first_rows(s), :], r[n_mem:]], axis=0)

        def part(j, p, i):
            return qkv[j][:, (3 * p + i) * dh:(3 * p + i + 1) * dh]

        def scores(j):
            for p in range(2):
                sc = _matmul_nt(part(j, p, 0), part(j, p, 1).astype(BF16)) * scale
                sc = jnp.where(visible, sc, MASKED)
                e = jnp.exp(sc - jnp.max(sc, axis=-1, keepdims=True))
                probs[j, p] = e / jnp.sum(e, axis=-1, keepdims=True)

        def mix(j):
            for p in range(2):
                heads[2 * j + p] = _matmul(probs[j, p], part(j, p, 2).astype(BF16))

        def out_proj(quarter):
            h0, h1 = quarter * n_pair // 2, (quarter + 1) * n_pair // 2
            o = jnp.concatenate([heads[h] for h in range(h0, h1)], axis=1)
            return _matmul(o, _weights(wo[h0 * dh // 2:h1 * dh // 2, :]))

        for j in range(n_pair):
            project(j)
            if j >= 1:
                scores(j - 1)
            if j >= 2:
                mix(j - 2)
        acc[...] = out_proj(0)
        scores(n_pair - 1)
        mix(n_pair - 2)
        fillers[0]()
        acc[...] += out_proj(1)
        mix(n_pair - 1)
        fillers[1]()
        acc[...] += out_proj(2)
        fillers[2]()
        o = acc[...] + out_proj(3)

        out_v[s] = ((x_v[s].astype(F32) + o[n_mem:]) + normalised(s)).astype(BF16)
        return o[:n_mem]

    def write_group(group, valid):
        for u in range(STEP_UNROLL):
            s = group * STEP_UNROLL + u
            pl.when(valid & (s != routed[0][0]) & (s != routed[1][0]))(out_copy(s).start)

    def steps(group, carry):
        @pl.when(group == ffn_start)
        def _():
            for c in ffn_copies:
                c.wait()

        pieces = ffn_pieces(group)
        assert len(pieces) == 3 * STEP_UNROLL
        memory = mem[...]
        for u in range(STEP_UNROLL):
            memory = step(group * STEP_UNROLL + u, memory, pieces[3 * u:3 * u + 3])
            if u == 0:
                write_group(jnp.maximum(group - 1, 0), group > 0)
        mem[...] = memory
        return carry

    lax.fori_loop(0, n_group, steps, 0)
    write_group(n_group - 1, True)

    y = y_acc[...] * gate[:, :1]
    for c, (s, r) in enumerate(routed):
        upd = jnp.where(seg_row == r, y[c:c + 1], 0.0)
        out_v[s] = (out_v[s].astype(F32) + upd).astype(BF16)
    out_copy(routed[0][0]).start()
    pl.when(routed[1][0] != routed[0][0])(out_copy(routed[1][0]).start)
    pltpu.make_async_copy(out_v, out_hbm, sem_out.at[0]).wait()


@functools.partial(jax.jit, static_argnames=("A_seg_len",))
def pallas_parallel_sum__memory_aug_recurrent_mem_tr__moe_arch_mod__prompt_kernel(
    A_x: jax.Array,
    A_mem0: jax.Array,
    A_Wq: jax.Array,
    A_Wk: jax.Array,
    A_Wv: jax.Array,
    A_Wo: jax.Array,
    A_seg_len: int,
    B_x: jax.Array,
    B_w_r: jax.Array,
    B_w_gate: jax.Array,
    B_w_up: jax.Array,
    B_w_down: jax.Array,
):
    del B_x
    batch, n_tok, dm = A_x.shape
    _, n_head, dh = A_Wq.shape
    n_mem = A_mem0.shape[1]
    seg = A_seg_len
    n_seg = n_tok // seg
    n_pair = n_head // 2
    ff = B_w_gate.shape[1]
    assert batch == 1 and n_mem == 8 and dh == 128 and seg % 16 == 0 and n_tok == n_seg * seg
    assert n_pair % PAIR_GROUP == 0 and n_seg % n_pair == 0
    assert n_seg % STEP_UNROLL == 0 and ff % FF_CHUNK == 0

    hbm = pl.BlockSpec(memory_space=pl.ANY)
    out = pl.pallas_call(
        _kernel,
        out_shape=jax.ShapeDtypeStruct((n_seg, seg, dm), A_x.dtype),
        in_specs=[hbm] * 10,
        out_specs=hbm,
        scratch_shapes=[
            pltpu.VMEM((n_seg, seg, dm), BF16),
            pltpu.VMEM((n_seg * PRE, dm), F32),
            pltpu.VMEM((n_seg, seg - PRE, dm), F32),
            pltpu.VMEM((n_pair, 3, dm, dh), U32),
            pltpu.VMEM((n_pair, dm // 2, 6 * dh), U32),
            pltpu.VMEM((n_head * dh // 2, dm), U32),
            pltpu.VMEM((n_pair, n_seg * PRE, 6 * dh), F32),
            pltpu.VMEM((n_mem, dm), F32),
            pltpu.VMEM((n_mem + seg, dm), F32),
            pltpu.VMEM((n_mem + seg - PRE, 6 * dh), F32),
            pltpu.VMEM((n_seg, seg, dm), BF16),
            pltpu.VMEM((8, dm), F32),
            pltpu.VMEM((dm // 2, ff + FF_CHUNK), U32),
            pltpu.VMEM((dm // 2, ff + FF_CHUNK), U32),
            pltpu.VMEM(((ff + FF_CHUNK) // 2, dm), U32),
            pltpu.VMEM((8, dm), F32),
            pltpu.VMEM((8, dm), F32),
            pltpu.VMEM((n_mem, dm), BF16),
            pltpu.VMEM((2, 8, FF_CHUNK), F32),
            pltpu.VMEM((8, FF_CHUNK), F32),
            pltpu.VMEM((NUM_ROUTED, 8, 128), F32),
            pltpu.VMEM((NUM_ROUTED, 8, 128), jnp.int32),
            pltpu.VMEM((8, 128), F32),
            pltpu.VMEM((dm,), BF16),
            pltpu.SemaphoreType.DMA((3 * n_pair + 8 + n_pair // PAIR_GROUP,)),
            pltpu.SemaphoreType.DMA((1,)),
        ],
        compiler_params=pltpu.CompilerParams(
            vmem_limit_bytes=126 * 1024 * 1024,
            flags={"XLA_TPU_EVENLY_DISTRIBUTE_CRITICAL_NODES": True},
        ),
        name="rmt_mod_fused",
    )(
        A_x.reshape(n_seg, seg, dm),
        A_mem0.reshape(n_mem, dm),
        A_Wq,
        A_Wk,
        A_Wv,
        A_Wo.reshape(n_head * dh, dm),
        B_w_r,
        B_w_gate,
        B_w_up,
        B_w_down,
    )
    return out.reshape(batch, n_tok, dm)
```
